```python
import os as _os
_os.environ.setdefault("JAX_PLATFORMS", "cpu")
import jax
import jax.numpy as jnp

def _softmax(x, axis=-1):
    return jax.nn.softmax(x, axis=axis)
def _gelu(x):
    return jax.nn.gelu(x, approximate=True)
def _silu(x):
    return jax.nn.silu(x)
def _sigmoid(x):
    return jax.nn.sigmoid(x)
def _layernorm(x, axis=-1, eps=1e-5):
    m = jnp.mean(x, axis=axis, keepdims=True)
    v = jnp.var(x, axis=axis, keepdims=True)
    return (x - m) / jnp.sqrt(v + eps)
def _scatter_add(tgt, idx, src, axis=0):
    return tgt.at[idx].add(src)
def _segment_sum(src, seg, n):
    return jax.ops.segment_sum(src, seg, n)
class _Rng:
    def __init__(self, key):
        self._k = key
    def _next(self):
        self._k, sub = jax.random.split(self._k)
        return sub
    def normal(self, shape):
        return jax.random.normal(self._next(), shape, dtype=jnp.bfloat16)
    def randint(self, lo, hi, shape):
        return jax.random.randint(self._next(), shape, lo, hi, dtype=jnp.int32)
    def uniform(self, shape, lo=0.0, hi=1.0):
        return jax.random.uniform(self._next(), shape, jnp.bfloat16, lo, hi)
    def permutation(self, n):
        return jax.random.permutation(self._next(), n)


kernel_name = 'interleave_layers__ssm_conv_h3__geglu_ffn__prompt'

def setup_inputs():
    _rng = _Rng(jax.random.key(int.from_bytes(__import__("os").urandom(4), "little")))
    _w = (lambda a: (lambda t: t.astype(jnp.bfloat16) if jnp.issubdtype(t.dtype, jnp.floating) else t)(jnp.asarray(a)))
    def _A_setup():
        B, S, D = 1, 2048, 448
        ks = 4
        return {
            "q": _w((lambda *s: _rng.normal(s) * 0.05)(B, S, D)),
            "k": _w((lambda *s: _rng.normal(s) * 0.8)(B, S, D)),
            "v": _w((lambda *s: _rng.normal(s) * 0.8)(B, S, D)),
            "shift_k": _w((lambda *s: _rng.normal(s) * 0.8)(D, ks) * 0.5),
            "ssm_k": _w((lambda *s: _rng.normal(s) * 0.8)(D, S) * (1.0 / S ** 0.5)),
            "ssm_D": _w((lambda *s: _rng.normal(s) * 0.8)(D)),
        }
    _A_in = _A_setup()

    def _B_setup():
        B, S, D, F = 1, 2048, 448, 1792
        return {
            "x": _w((lambda *s: _rng.normal(s) * 0.05)(B, S, D)),
            "w_gate": _w((lambda *s: _rng.normal(s) * 0.1)(D, F)),
            "w_up": _w((lambda *s: _rng.normal(s) * 0.1)(D, F)),
            "w_down": _w((lambda *s: _rng.normal(s) * 0.1)(F, D)),
        }
    _B_in = _B_setup()

    return {
        "A_q": _A_in["q"],
        "A_k": _A_in["k"],
        "A_v": _A_in["v"],
        "A_shift_k": _A_in["shift_k"],
        "A_ssm_k": _A_in["ssm_k"],
        "A_ssm_D": _A_in["ssm_D"],
        "B_x": _B_in["x"],
        "B_w_gate": _B_in["w_gate"],
        "B_w_up": _B_in["w_up"],
        "B_w_down": _B_in["w_down"],
    }

def reference(A_q, A_k, A_v, A_shift_k, A_ssm_k, A_ssm_D, B_x, B_w_gate, B_w_up, B_w_down):
    def _A_ref(q, k, v, shift_k, ssm_k, ssm_D):
        B, S, D = q.shape
        ks = shift_k.shape[-1]
        k_pad = jnp.pad(k, ((0, 0), (ks - 1, 0), (0, 0)))
        k_shift = jnp.zeros_like(k)
        for t in range(ks):
            k_shift = k_shift + k_pad[:, t:t + S, :] * shift_k[:, ks - 1 - t][None, None, :]
        kv = k_shift * v
        L = 2 * S
        kv_pad = jnp.pad(kv, ((0, 0), (0, S), (0, 0)))
        kf_pad = jnp.pad(ssm_k, ((0, 0), (0, S)))
        kv_f = (lambda x, axes=(-2,-1): jnp.fft.rfft2(x.astype(jnp.float32), axes=axes))(kv_pad[:, None, :, :], axes=(1, 2))
        kf_f = (lambda x, axes=(-2,-1): jnp.fft.rfft2(x.astype(jnp.float32), axes=axes))(kf_pad[:, None, :], axes=(1, 2))
        kf_f = (lambda x, *d: x.transpose(*d))(kf_f, 1, 2, 0)
        y_f = kv_f * kf_f[None, :, :, :]
        y = (lambda x, s, axes=(-2,-1): jnp.fft.irfft2(x, s=s, axes=axes).astype(jnp.bfloat16))(y_f, (1, L), axes=(1, 2))[:, 0, :S, :]
        y = y + kv * ssm_D[None, None, :]
        return q * y

    def _B_ref(x, w_gate, w_up, w_down):
        return (_gelu(x @ w_gate) * (x @ w_up)) @ w_down

    x = A_q
    x = x + _A_ref(_layernorm(x, axis=-1), A_k, A_v, A_shift_k, A_ssm_k, A_ssm_D)
    x = x + _B_ref(_layernorm(x, axis=-1), B_w_gate, B_w_up, B_w_down)
    x = x + _A_ref(_layernorm(x, axis=-1), A_k, A_v, A_shift_k, A_ssm_k, A_ssm_D)
    x = x + _B_ref(_layernorm(x, axis=-1), B_w_gate, B_w_up, B_w_down)
    return x
```

```python
import functools
import math
import jax
import jax.numpy as jnp
from jax import lax
from jax.experimental import pallas as pl
from jax.experimental.pallas import tpu as pltpu

S, D, F = 2048, 448, 1792
B = 128
NB = S // B
TM = 256
f32 = jnp.float32
bf16 = jnp.bfloat16


def _dft_mats():
    n = lax.broadcasted_iota(jnp.int32, (B, B), 0)
    f = lax.broadcasted_iota(jnp.int32, (B, B), 1)
    m = ((2 * f + 1) * n) & 511
    m = jnp.where(m >= 256, m - 512, m)
    ang = m.astype(f32) * (math.pi / 256.0)
    ffwd = jnp.concatenate([jnp.cos(ang), -jnp.sin(ang)], axis=1).astype(bf16)
    fi = lax.broadcasted_iota(jnp.int32, (B, B), 0)
    a = lax.broadcasted_iota(jnp.int32, (B, B), 1) + B
    m2 = ((2 * fi + 1) * a) & 511
    m2 = jnp.where(m2 >= 256, m2 - 512, m2)
    ang2 = m2.astype(f32) * (math.pi / 256.0)
    finv = (jnp.concatenate([jnp.cos(ang2), -jnp.sin(ang2)], axis=0) * (2.0 / 256.0)).astype(bf16)
    return ffwd, finv


def _ln(x):
    m = jnp.mean(x, axis=0, keepdims=True)
    xc = x - m
    v = jnp.mean(xc * xc, axis=0, keepdims=True)
    return xc * lax.rsqrt(v + 1e-5)


def _gelu(x):
    c = math.sqrt(2.0 / math.pi)
    return 0.5 * x * (1.0 + jnp.tanh(c * (x + 0.044715 * (x * x * x))))


def kernel(q_ref, k_ref, v_ref, sk_ref, h_ref, d_ref, wg_ref, wu_ref, wd_ref, o_ref,
           wgT, wuT, y_scr, u_scr, g_scr):
    @pl.when(pl.program_id(0) == 0)
    def _():
        wgT[...] = wg_ref[...].T
        wuT[...] = wu_ref[...].T
        ffwd, finv = _dft_mats()
        sk = sk_ref[...].astype(f32)
        dv = d_ref[...].astype(f32).reshape(1, D)
        ct = jnp.concatenate([sk, dv, jnp.zeros((3, D), f32)], axis=0).T
        k = k_ref[...].astype(f32)
        lane = lax.broadcasted_iota(jnp.int32, (D, S), 1)
        ks = k * ct[:, 0:1]
        for j in range(1, 4):
            kj = jnp.where(lane >= j, pltpu.roll(k, j, 1), 0.0)
            ks = ks + kj * ct[:, j:j + 1]
        kv = (ks * v_ref[...].astype(f32)).astype(bf16)
        y_scr[...] = kv.astype(f32) * ct[:, 4:5]
        sgn = 1.0 - 2.0 * (lax.broadcasted_iota(jnp.int32, (1, B), 1) & 1).astype(f32)
        hprev = None
        for i in range(NB):
            U = jnp.dot(kv[:, i * B:(i + 1) * B], ffwd, preferred_element_type=f32)
            ar, ai = U[:, :B], U[:, B:]
            u_scr[0, i] = ar + ai
            u_scr[1, i] = ar
            u_scr[2, i] = ai
            H = jnp.dot(h_ref[:, i * B:(i + 1) * B], ffwd, preferred_element_type=f32)
            hr, hi = H[:, :B], H[:, B:]
            br, bi = sgn * hi, -sgn * hr
            if hprev is not None:
                br = br + hprev[0]
                bi = bi + hprev[1]
            hprev = (hr, hi)
            g_scr[0, i] = br
            g_scr[1, i] = bi - br
            g_scr[2, i] = br + bi

        def rows(r, carry):
            r0 = pl.multiple_of(r * 8, 8)
            ks_ = []
            for t in range(3):
                us = [u_scr[t, j, pl.ds(r0, 8), :] for j in range(NB)]
                gs = [g_scr[t, j, pl.ds(r0, 8), :] for j in range(NB)]
                outs = []
                for i in range(NB):
                    acc = gs[i] * us[0]
                    for j in range(1, i + 1):
                        acc = acc + gs[i - j] * us[j]
                    outs.append(acc)
                ks_.append(outs)
            for i in range(NB):
                u_scr[1, i, pl.ds(r0, 8), :] = ks_[0][i] - ks_[2][i]
                u_scr[2, i, pl.ds(r0, 8), :] = ks_[0][i] + ks_[1][i]
            return carry
        lax.fori_loop(0, D // 8, rows, 0)

        for i in range(NB):
            Y = jnp.concatenate([u_scr[1, i], u_scr[2, i]], axis=1).astype(bf16)
            yi = jnp.dot(Y, finv, preferred_element_type=f32)
            y_scr[:, i * B:(i + 1) * B] = y_scr[:, i * B:(i + 1) * B] + yi

    i = pl.program_id(0)
    t0 = pl.multiple_of(i * TM, TM)
    y = y_scr[:, pl.ds(t0, TM)]
    x = q_ref[...].astype(f32)
    for _ in range(2):
        x = x + _ln(x) * y
        xn = _ln(x).astype(bf16)
        g = jnp.dot(wgT[...], xn, preferred_element_type=f32)
        u = jnp.dot(wuT[...], xn, preferred_element_type=f32)
        hh = (_gelu(g) * u).astype(bf16)
        x = x + jnp.dot(wd_ref[...], hh, preferred_element_type=f32)
    o_ref[...] = x.astype(o_ref.dtype)


@jax.jit
def pallas_interleave_layers__ssm_conv_h3__geglu_ffn__prompt_kernel(A_q, A_k, A_v, A_shift_k, A_ssm_k, A_ssm_D, B_x, B_w_gate, B_w_up, B_w_down):
    full = lambda shape: pl.BlockSpec(shape, lambda i: (0,) * len(shape))
    out = pl.pallas_call(
        kernel,
        grid=(S // TM,),
        in_specs=[
            pl.BlockSpec((D, TM), lambda i: (0, i)),
            full((D, S)), full((D, S)), full((4, D)), full((D, S)), full((D,)),
            full((D, F)), full((D, F)), full((D, F)),
        ],
        out_specs=pl.BlockSpec((D, TM), lambda i: (0, i)),
        out_shape=jax.ShapeDtypeStruct((D, S), bf16),
        scratch_shapes=[
            pltpu.VMEM((F, D), bf16), pltpu.VMEM((F, D), bf16),
            pltpu.VMEM((D, S), f32),
            pltpu.VMEM((3, NB, D, B), f32), pltpu.VMEM((3, NB, D, B), f32),
        ],
        compiler_params=pltpu.CompilerParams(dimension_semantics=("arbitrary",), vmem_limit_bytes=110 * 1024 * 1024),
    )(A_q[0].T, A_k[0].T, A_v[0].T, A_shift_k.T, A_ssm_k, A_ssm_D, B_w_gate, B_w_up, B_w_down.T)
    return out.T[None]
```

```python
import functools
import math
import jax
import jax.numpy as jnp
from jax import lax
from jax.experimental import pallas as pl
from jax.experimental.pallas import tpu as pltpu

S, D, F = 2048, 448, 1792
B = 128
NB = S // B
PW = 2 * B
NP = S // PW
TM = 512
TH = TM // 2
KH = D // 2
FH = F // 2
NCH = F // PW
RC = 32
UC = 16
f32 = jnp.float32
bf16 = jnp.bfloat16
u32 = jnp.uint32

UNITS = (
    ((5, 1), (4, 0), (4, 4), (5, 2), (5, 3), (5, 4)),
    ((6, 1), (5, 0), (5, 5), (6, 2), (6, 3), (6, 4)),
    ((7, 1), (6, 0), (6, 5), (6, 6), (7, 2), (7, 3)),
    ((8, 7), (7, 0), (7, 4), (7, 5), (7, 6), (7, 7)),
)
NSLOT = 6


def _dft_mats():
    n = lax.broadcasted_iota(jnp.int32, (B, B), 0)
    f = lax.broadcasted_iota(jnp.int32, (B, B), 1)
    m = ((2 * f + 1) * n) & 511
    m = jnp.where(m >= 256, m - 512, m)
    ang = m.astype(f32) * (math.pi / 256.0)
    ffwd = jnp.concatenate([jnp.cos(ang), -jnp.sin(ang)], axis=1).astype(bf16)
    m2 = ((2 * n + 1) * (f + B)) & 511
    m2 = jnp.where(m2 >= 256, m2 - 512, m2)
    ang2 = m2.astype(f32) * (math.pi / 256.0)
    finv = (jnp.concatenate([jnp.cos(ang2), -jnp.sin(ang2)], axis=0) * (2.0 / 256.0)).astype(bf16)
    return ffwd, finv


def _ln(x):
    m = jnp.mean(x, axis=0, keepdims=True)
    xc = x - m
    v = jnp.mean(xc * xc, axis=0, keepdims=True)
    return xc * lax.rsqrt(v + 1e-5)


def _gelu(x):
    c = math.sqrt(2.0 / math.pi)
    return 0.5 * x * (1.0 + jnp.tanh(c * (x + 0.044715 * (x * x * x))))


def _acombos(a11, a12, a21, a22):
    return [a11 + a22, a21 + a22, a11, a22, a11 + a12, a21 - a11, a12 - a22]


def _pack(x):
    return pltpu.bitcast(x.astype(bf16), u32)


def _unpack(x):
    return pltpu.bitcast(x, bf16)


def _dot(a, b):
    return jnp.dot(a, b, preferred_element_type=f32)


def _act(c):
    rows = c.shape[0] // 2
    c = c.reshape(rows // 16, 2, 16, TH)
    return (_gelu(c[:, 0]) * c[:, 1]).reshape(rows, TH)


def kernel(q_hbm, k_hbm, v_hbm, sk_hbm, h_hbm, d_hbm, wg_hbm, wu_hbm, wd_hbm, o_hbm,
           q_v, k_v, v_v, h_v, wg_v, wu_v, wd_v, sk_v, d_v, agu, ad, ffwd_v, finv_v, coef,
           u_s, g_s, hp_s, ya_s, y_s, o_v, kv_s, hq, xb, bc_s, tab, par, in_sem, w_sem, o_sem, s_sem):

    def in_copies(m):
        c0 = m * PW if isinstance(m, int) else pl.multiple_of(m * PW, PW)
        return [pltpu.make_async_copy(src.at[:, pl.ds(c0, PW)], dst.at[m], in_sem.at[4 * m + i])
                for i, (src, dst) in enumerate(((k_hbm, k_v), (v_hbm, v_v), (h_hbm, h_v)))]

    def q_copies(ms):
        return [pltpu.make_async_copy(q_hbm.at[:, pl.ds(m * PW, PW)], q_v.at[m], in_sem.at[4 * m + 3]) for m in ms]

    def gu_copies(c):
        return [pltpu.make_async_copy(src.at[:, pl.ds(c * PW, PW)], dst.at[:, pl.ds(c * PW, PW)], w_sem.at[2 * c + i])
                for i, (src, dst) in enumerate(((wg_hbm, wg_v), (wu_hbm, wu_v)))]

    def d_copies():
        return [pltpu.make_async_copy(wd_hbm, wd_v, w_sem.at[2 * NCH])]

    def small_copies():
        return [pltpu.make_async_copy(sk_hbm, sk_v, s_sem.at[0]), pltpu.make_async_copy(d_hbm, d_v, s_sem.at[1])]

    def out_copy(b):
        return pltpu.make_async_copy(o_v.at[b], o_hbm.at[:, pl.ds(b * TM, TM)], o_sem.at[b])

    def start(cps):
        for cp in cps:
            cp.start()

    def wait(cps):
        for cp in cps:
            cp.wait()

    start(small_copies())
    start(in_copies(0))
    for n in range(len(UNITS)):
        for s in range(NSLOT):
            tab[(n * NSLOT + s) * 2] = UNITS[n][s][0]
            tab[(n * NSLOT + s) * 2 + 1] = UNITS[n][s][1]

    for i in range(8):
        par[i] = i // 4
    par[8] = 0
    par[9] = 0
    ffwd, finv = _dft_mats()
    ffwd_v[...] = pltpu.bitcast(ffwd, u32)
    finv_v[...] = pltpu.bitcast(finv, u32)
    zero_blk = jnp.zeros((D, B), f32)
    for t in range(3):
        g_s[t, 0] = zero_blk
    wait(small_copies())
    start(in_copies(1) + q_copies((0, 1)) + gu_copies(0) + gu_copies(1))
    sk = sk_v[...].astype(f32)
    dv = d_v[...].astype(f32).reshape(1, D)
    for j in range(5):
        row = sk[j:j + 1] if j < 4 else dv
        coef[j] = jnp.broadcast_to(row, (B, D)).T

    def conv_h(m):
        T = [_dot(h_v[m, :, c * B:(c + 1) * B], _unpack(ffwd_v[...])) for c in range(2)]
        sgn = 1.0 - 2.0 * (lax.broadcasted_iota(jnp.int32, (1, B), 1) & 1).astype(f32)
        first = isinstance(m, int) and m == 0
        if not first:
            hr_p, hi_p = hp_s[0], hp_s[1]
        for c in range(2):
            hr, hi = T[c][:, :B], T[c][:, B:]
            br = sgn * hi
            bi = -sgn * hr
            if not (first and c == 0):
                br = br + hr_p
                bi = bi + hi_p
            g_s[0, 2 * m + c + 1] = br
            g_s[1, 2 * m + c + 1] = bi - br
            g_s[2, 2 * m + c + 1] = br + bi
            hr_p, hi_p = hr, hi
        hp_s[0] = hr_p
        hp_s[1] = hi_p

    def conv_u(m):
        lane = lax.broadcasted_iota(jnp.int32, (RC // 2, B), 1)
        for r in range(D // RC):
            rs = slice(r * RC, (r + 1) * RC)
            if isinstance(m, int) and m == 0:
                halo = jnp.zeros((RC // 2, B), u32)
            else:
                halo = pltpu.bitcast(k_v[m - 1, rs, B:PW], u32)
            tiles = [halo, pltpu.bitcast(k_v[m, rs, 0:B], u32), pltpu.bitcast(k_v[m, rs, B:PW], u32)]
            rolled = [[pltpu.roll(t, j, 1) for t in tiles] for j in range(1, 4)]
            for c in range(2):
                ks = _unpack(tiles[c + 1]).astype(f32) * coef[0, rs]
                for j in range(1, 4):
                    kj = jnp.where(lane >= j, rolled[j - 1][c + 1], rolled[j - 1][c])
                    ks = ks + _unpack(kj).astype(f32) * coef[j, rs]
                kv = (ks * v_v[m, rs, c * B:(c + 1) * B].astype(f32)).astype(bf16)
                y_s[2 * m + c, rs] = kv.astype(f32) * coef[4, rs]
                kv_s[c, r * RC // 2:(r + 1) * RC // 2] = pltpu.bitcast(kv, u32)

    def conv_u_dot(m):
        T = [_dot(_unpack(kv_s[c]), _unpack(ffwd_v[...])) for c in range(2)]
        for c in range(2):
            ar, ai = T[c][:, :B], T[c][:, B:]
            u_s[0, 2 * m + c] = ar + ai
            u_s[1, 2 * m + c] = ar
            u_s[2, 2 * m + c] = ai

    def conv_unit(I, J, init=False):
        dl = 2 * (I - J)
        diag = isinstance(dl, int) and dl == 0
        for r in range(D // UC):
            rs = pl.ds(r * UC, UC)
            k0, k1 = [], []
            for t in range(3):
                gb, gc = g_s[t, dl + 1, rs], g_s[t, dl + 2, rs]
                u0, u1 = u_s[t, 2 * J, rs], u_s[t, 2 * J + 1, rs]
                k0.append(gb * u0 if diag else gb * u0 + g_s[t, dl, rs] * u1)
                k1.append(gc * u0 + gb * u1)
            for a, ks in enumerate((k0, k1)):
                re, im = ks[0] - ks[2], ks[0] + ks[1]
                if not init:
                    re = ya_s[0, 2 * I + a, rs] + re
                    im = ya_s[1, 2 * I + a, rs] + im
                ya_s[0, 2 * I + a, rs] = re
                ya_s[1, 2 * I + a, rs] = im

    def conv_inverse(m):
        yi = [_dot(jnp.concatenate([ya_s[0, 2 * m + c], ya_s[1, 2 * m + c]], axis=1).astype(bf16),
                   _unpack(finv_v[...])) for c in range(2)]
        for c in range(2):
            y_s[2 * m + c] = y_s[2 * m + c] + yi[c]

    def prep_gu(c):
        for i, w in enumerate((wg_v, wu_v)):
            wt1 = w[0:KH, c * PW:(c + 1) * PW].T.astype(f32)
            wt2 = w[KH:D, c * PW:(c + 1) * PW].T.astype(f32)
            cs = _acombos(wt1[:B], wt2[:B], wt1[B:], wt2[B:])
            for p in range(7):
                agu[p, c * 8:(c + 1) * 8, i] = _pack(cs[p]).reshape(8, 8, KH)

    def prep_d():
        for c in range(NCH):
            w = wd_v[:, c * PW:(c + 1) * PW].astype(f32)
            cs = _acombos(w[:KH, :B], w[:KH, B:], w[KH:, :B], w[KH:, B:])
            for p in range(7):
                ad[p, :, c * B:(c + 1) * B] = _pack(cs[p])

    def item_block(n):
        return 2 * (n // 4) + n % 2

    def head(n):
        static = isinstance(n, int)
        blk = item_block(n) if static else jnp.minimum(item_block(n), S // TM - 1)
        for c in range(TM // B):
            slot = par[(n % 2) * 4 + c]
            rs = slice((c // 2) * D, (c // 2 + 1) * D)
            cs = slice((c % 2) * B, (c % 2 + 1) * B)
            xr = lambda: xb[2 + slot, rs, cs]
            mu = jnp.mean(xr(), axis=0, keepdims=True)
            xc = xr() - mu
            rstd = lax.rsqrt(jnp.mean(xc * xc, axis=0, keepdims=True) + 1e-5)
            x0 = xr()
            x1 = x0 + (x0 - mu) * rstd * y_s[4 * blk + c]
            xb[2 + slot, rs, cs] = x1
            mu = jnp.mean(x1, axis=0, keepdims=True)
            xc = xr() - mu
            rstd = lax.rsqrt(jnp.mean(xc * xc, axis=0, keepdims=True) + 1e-5)
            xb[slot, rs, cs] = (xr() - mu) * rstd

    def load_q(slot, blk):
        for hf in range(2):
            xb[2 + slot, hf * D:(hf + 1) * D] = q_v[2 * blk + hf].astype(f32)

    def b_operand(slot, p):
        b11 = lambda: xb[slot, 0:KH]
        b21 = lambda: xb[slot, KH:D]
        b12 = lambda: xb[slot, D:D + KH]
        b22 = lambda: xb[slot, D + KH:2 * D]
        return (lambda: b11() + b22(), b11, lambda: b12() - b22(), lambda: b21() - b11(), b22,
                lambda: b11() + b12(), lambda: b21() + b22())[p]().astype(bf16)

    def down_and_tail(n, mid):
        slot = n % 2
        blk = item_block(n)

        def Ad(p):
            return _unpack(ad[p])

        mid()
        head(n + 1)
        d4 = _dot(Ad(3), (hq[2] - hq[0]).astype(bf16))
        d6 = _dot(Ad(5), (hq[0] + hq[1]).astype(bf16))
        d5 = _dot(Ad(4), hq[3].astype(bf16))
        d1 = _dot(Ad(0), (hq[0] + hq[3]).astype(bf16))
        top = jnp.where(par[8] == 1, xb[par[9], 0:16], hq[0, 0:16])
        d2 = _dot(Ad(1), jnp.concatenate([top, hq[0, 16:]], axis=0).astype(bf16))
        d3 = _dot(Ad(2), (hq[1] - hq[3]).astype(bf16))
        d7 = _dot(Ad(6), (hq[2] + hq[3]).astype(bf16))
        last = (n // 2) % 2 == 1
        for (hf, kh, o) in ((0, 1, d2 + d4), (1, 0, d3 + d5), (1, 1, d1 - d2 + d3 + d6), (0, 0, d1 + d4 - d5 + d7)):
            rs = slice(hf * D + kh * KH, hf * D + (kh + 1) * KH)
            xo = xb[2 + slot, rs] + o
            if isinstance(n, int):
                xb[2 + slot, rs] = xo
            else:
                o_v[blk, kh * KH:(kh + 1) * KH, hf * TH:(hf + 1) * TH] = xo.astype(bf16)
                nb = jnp.minimum(blk + 2, S // TM - 1)
                qn = q_v[2 * nb + hf, kh * KH:(kh + 1) * KH].astype(f32)
                xb[2 + slot, rs] = jnp.where(last, qn, xo)

    wait(in_copies(0))
    start(gu_copies(2) + in_copies(2))
    conv_h(0)
    conv_u(0)
    conv_u_dot(0)
    conv_unit(0, 0, init=True)
    conv_inverse(0)
    wait(in_copies(1))
    start(gu_copies(3) + gu_copies(4))
    conv_h(1)
    conv_u(1)
    conv_u_dot(1)
    wait(gu_copies(0) + q_copies((0, 1)))
    conv_unit(1, 0, init=True)
    conv_unit(1, 1)
    conv_inverse(1)
    prep_gu(0)
    load_q(0, 0)
    head(0)
    for p in range(7):
        bc_s[p] = pltpu.bitcast(b_operand(0, p), u32)

    def products(c):
        def mm(p):
            return _dot(_unpack(agu[p, c * 8:(c + 1) * 8].reshape(B, KH)), _unpack(bc_s[p]))
        rs = slice(c * B, (c + 1) * B)
        m2, m4 = mm(1), mm(3)
        hq[2, rs] = _act(m2 + m4)
        m5, m3 = mm(4), mm(2)
        hq[1, rs] = _act(m3 + m5)
        m1, m7 = mm(0), mm(6)
        hq[0, rs] = _act(m1 + m4 - m5 + m7)
        m6 = mm(5)
        hq[3, rs] = _act(m1 - m2 + m3 + m6)

    wait(gu_copies(1) + gu_copies(2))
    start(in_copies(3) + gu_copies(5) + gu_copies(6))
    products(0)
    prep_gu(1)
    products(1)
    prep_gu(2)
    wait(gu_copies(3) + gu_copies(4) + in_copies(2))
    start(d_copies() + q_copies((2, 3)))
    conv_h(2)
    products(2)
    prep_gu(3)
    conv_u(2)
    conv_u_dot(2)
    products(3)
    prep_gu(4)
    conv_unit(2, 0, init=True)
    conv_unit(2, 1)
    conv_unit(2, 2)
    wait(gu_copies(5) + gu_copies(6) + in_copies(3))
    conv_h(3)
    products(4)
    prep_gu(5)
    conv_u(3)
    conv_u_dot(3)
    products(5)
    prep_gu(6)
    conv_unit(3, 1, init=True)
    conv_unit(3, 2)
    wait(d_copies() + q_copies((2, 3)))
    start(in_copies(4) + q_copies((4, 5, 6, 7)))
    products(6)
    prep_d()
    conv_unit(3, 0)
    conv_unit(3, 3)

    def mid0():
        load_q(1, 1)
        conv_inverse(2)
        conv_inverse(3)
        conv_unit(4, 1, init=True)
        conv_unit(4, 2)
        conv_unit(4, 3)
    down_and_tail(0, mid0)

    def body(n, with_conv):
        slot = n % 2
        m = n + 3

        def unit(s):
            if with_conv:
                i = ((n - 1) * NSLOT + s) * 2
                conv_unit(tab[i], tab[i + 1], init=(s == 0))

        def mm(p):
            return _dot(_unpack(agu[p].reshape(F // 2, KH)), b_operand(slot, p))

        if with_conv:
            wait(in_copies(m))

            @pl.when(m < NP - 1)
            def _():
                start(in_copies(jnp.minimum(m + 1, NP - 1)))
            conv_h(m)
        m2 = mm(1)
        m5 = mm(4)
        if with_conv:
            conv_u(m)
            conv_u_dot(m)
        m1 = mm(0)
        unit(0)
        unit(1)
        m4 = mm(3)
        hq[2] = _act(m2 + m4)
        unit(2)
        m3 = mm(2)
        hq[1] = _act(m3 + m5)
        unit(3)
        unit(4)
        unit(5)
        if with_conv:
            conv_inverse(m)
        m7 = mm(6)
        hq[0] = _act(m1 + m4 - m5 + m7)
        m6 = mm(5)
        hq[3] = _act(m1 - m2 + m3 + m6)
        down_and_tail(n, lambda: None)

        @pl.when((n // 2) % 2 == 1)
        def _():
            out_copy(item_block(n)).start()

    def body_conv(n, carry):
        body(n, True)
        return carry

    def body_plain(n, carry):
        body(n, False)
        return carry

    wait(q_copies((4, 5, 6, 7)))
    lax.fori_loop(1, 5, body_conv, 0)
    lax.fori_loop(5, 8, body_plain, 0)
    for b in range(S // TM):
        out_copy(b).wait()


@jax.jit
def pallas_interleave_layers__ssm_conv_h3__geglu_ffn__prompt_kernel(A_q, A_k, A_v, A_shift_k, A_ssm_k, A_ssm_D, B_x, B_w_gate, B_w_up, B_w_down):
    hbm = pl.BlockSpec(memory_space=pl.ANY)
    out = pl.pallas_call(
        kernel,
        in_specs=[hbm] * 9,
        out_specs=hbm,
        out_shape=jax.ShapeDtypeStruct((D, S), bf16),
        scratch_shapes=[
            pltpu.VMEM((NP, D, PW), bf16), pltpu.VMEM((NP, D, PW), bf16),
            pltpu.VMEM((NP, D, PW), bf16), pltpu.VMEM((NP, D, PW), bf16),
            pltpu.VMEM((D, F), bf16), pltpu.VMEM((D, F), bf16), pltpu.VMEM((D, F), bf16),
            pltpu.VMEM((4, D), bf16), pltpu.VMEM((D,), bf16),
            pltpu.VMEM((7, FH // 16, 2, 8, KH), u32), pltpu.VMEM((7, KH // 2, FH), u32),
            pltpu.VMEM((B // 2, 2 * B), u32), pltpu.VMEM((B, B), u32),
            pltpu.VMEM((5, D, B), f32),
            pltpu.VMEM((3, NB, D, B), f32), pltpu.VMEM((3, NB + 1, D, B), f32),
            pltpu.VMEM((2, D, B), f32), pltpu.VMEM((2, NB + 2, D, B), f32),
            pltpu.VMEM((NB, D, B), f32), pltpu.VMEM((S // TM, D, TM), bf16),
            pltpu.VMEM((2, D // 2, B), u32), pltpu.VMEM((4, FH, TH), f32), pltpu.VMEM((4, FH, TH), f32), pltpu.VMEM((7, KH // 2, TH), u32),
            pltpu.SMEM((len(UNITS) * NSLOT * 2,), jnp.int32), pltpu.SMEM((10,), jnp.int32),
            pltpu.SemaphoreType.DMA((4 * NP,)), pltpu.SemaphoreType.DMA((2 * NCH + 1,)),
            pltpu.SemaphoreType.DMA((S // TM,)), pltpu.SemaphoreType.DMA((2,)),
        ],
        compiler_params=pltpu.CompilerParams(vmem_limit_bytes=110 * 1024 * 1024),
    )(A_q[0].T, A_k[0].T, A_v[0].T, A_shift_k.T, A_ssm_k, A_ssm_D, B_w_gate, B_w_up, B_w_down.T)
    return out.T[None]
```

```python
import functools
import math
import jax
import jax.numpy as jnp
from jax import lax
from jax.experimental import pallas as pl
from jax.experimental.pallas import tpu as pltpu

S, D, F = 2048, 448, 1792
B = 128
NB = S // B
PW = 2 * B
NP = S // PW
TM = 512
TH = TM // 2
KH = D // 2
FH = F // 2
NCH = F // PW
RC = 32
UC = 16
f32 = jnp.float32
bf16 = jnp.bfloat16
u32 = jnp.uint32

UNITS = (
    ((5, 1), (4, 0), (4, 3), (4, 4), (5, 2), (5, 3)),
    ((6, 1), (5, 0), (5, 4), (5, 5), (6, 2), (6, 3)),
    ((7, 1), (6, 0), (6, 4), (6, 5), (6, 6), (7, 2)),
    ((7, 3), (7, 0), (7, 4), (7, 5), (7, 6), (7, 7)),
)
NSLOT = 6
PADN = 100
MULTI = False
UNITS0 = ((2, 0), (2, 1), (2, 2), (4, 2), (3, 1), (3, 2), (3, 0), (3, 3), (4, 1))


def _dft_mats():
    n = lax.broadcasted_iota(jnp.int32, (B, B), 0)
    f = lax.broadcasted_iota(jnp.int32, (B, B), 1)
    m = ((2 * f + 1) * n) & 511
    m = jnp.where(m >= 256, m - 512, m)
    ang = m.astype(f32) * (math.pi / 256.0)
    ffwd = jnp.concatenate([jnp.cos(ang), -jnp.sin(ang)], axis=1).astype(bf16)
    m2 = ((2 * n + 1) * (f + B)) & 511
    m2 = jnp.where(m2 >= 256, m2 - 512, m2)
    ang2 = m2.astype(f32) * (math.pi / 256.0)
    finv = (jnp.concatenate([jnp.cos(ang2), -jnp.sin(ang2)], axis=0) * (2.0 / 256.0)).astype(bf16)
    return ffwd, finv


def _ln(x):
    m = jnp.mean(x, axis=0, keepdims=True)
    xc = x - m
    v = jnp.mean(xc * xc, axis=0, keepdims=True)
    return xc * lax.rsqrt(v + 1e-5)


def _gelu(x):
    c = math.sqrt(2.0 / math.pi)
    return 0.5 * x * (1.0 + jnp.tanh(c * (x + 0.044715 * (x * x * x))))


def _acombos(a11, a12, a21, a22):
    return [a11 + a22, a21 + a22, a11, a22, a11 + a12, a21 - a11, a12 - a22]


def _pack(x):
    return pltpu.bitcast(x.astype(bf16), u32)


def _unpack(x):
    return pltpu.bitcast(x, bf16)


def _dot(a, b):
    return jnp.dot(a, b, preferred_element_type=f32)


def _act(c):
    rows = c.shape[0] // 2
    c = c.reshape(rows // 16, 2, 16, TH)
    return (_gelu(c[:, 0]) * c[:, 1]).reshape(rows, TH)


def kernel(q_hbm, k_hbm, v_hbm, sk_hbm, h_hbm, d_hbm, wg_hbm, wu_hbm, wd_hbm, o_hbm,
           q_v, k_v, v_v, h_v, wg_v, wu_v, wd_v, sk_v, d_v, agu, ad, ffwd_v, finv_v, coef,
           u_s, g_s, hp_s, ya_s, y_s, o_v, kv_s, hq, xb, bc_s, tab, par, in_sem, w_sem, o_sem, s_sem):

    def in_copies(m):
        c0 = m * PW if isinstance(m, int) else pl.multiple_of(m * PW, PW)
        return [pltpu.make_async_copy(src.at[:, pl.ds(c0, PW)], dst.at[m], in_sem.at[4 * m + i])
                for i, (src, dst) in enumerate(((k_hbm, k_v), (v_hbm, v_v), (h_hbm, h_v)))]

    def q_copies(ms):
        return [pltpu.make_async_copy(q_hbm.at[:, pl.ds(m * PW, PW)], q_v.at[m], in_sem.at[4 * m + 3]) for m in ms]

    def gu_copies(c):
        return [pltpu.make_async_copy(src.at[:, pl.ds(c * PW, PW)], dst.at[:, pl.ds(c * PW, PW)], w_sem.at[2 * c + i])
                for i, (src, dst) in enumerate(((wg_hbm, wg_v), (wu_hbm, wu_v)))]

    def d_copies():
        return [pltpu.make_async_copy(wd_hbm, wd_v, w_sem.at[2 * NCH])]

    def small_copies():
        return [pltpu.make_async_copy(sk_hbm, sk_v, s_sem.at[0]), pltpu.make_async_copy(d_hbm, d_v, s_sem.at[1])]

    def out_copy(b):
        return pltpu.make_async_copy(o_v.at[b], o_hbm.at[:, pl.ds(b * TM, TM)], o_sem.at[b])

    def start(cps):
        for cp in cps:
            cp.start()

    def wait(cps):
        for cp in cps:
            cp.wait()

    start(small_copies())
    start(in_copies(0) + q_copies((0,)))
    for n in range(len(UNITS)):
        for s in range(NSLOT):
            tab[(n * NSLOT + s) * 2] = UNITS[n][s][0]
            tab[(n * NSLOT + s) * 2 + 1] = UNITS[n][s][1]
    for s, (i, j) in enumerate(UNITS0):
        tab[(len(UNITS) * NSLOT + s) * 2] = i
        tab[(len(UNITS) * NSLOT + s) * 2 + 1] = j

    for i in range(8):
        par[i] = i // 4
    par[8] = 0
    par[9] = 0
    for c in range(NCH):
        par[10 + c] = c
    ffwd, finv = _dft_mats()
    ffwd_v[...] = pltpu.bitcast(ffwd, u32)
    finv_v[...] = pltpu.bitcast(finv, u32)
    zero_blk = jnp.zeros((D, B), f32)
    for t in range(3):
        g_s[t, 0] = zero_blk
    wait(small_copies())
    start(gu_copies(0) + in_copies(1) + q_copies((1,)))
    sk = sk_v[...].astype(f32)
    dv = d_v[...].astype(f32).reshape(1, D)
    for j in range(5):
        row = sk[j:j + 1] if j < 4 else dv
        coef[j] = jnp.broadcast_to(row, (B, D)).T

    def conv_h(m):
        T = [_dot(h_v[m, :, c * B:(c + 1) * B], _unpack(ffwd_v[...])) for c in range(2)]
        sgn = 1.0 - 2.0 * (lax.broadcasted_iota(jnp.int32, (1, B), 1) & 1).astype(f32)
        first = isinstance(m, int) and m == 0
        if not first:
            hr_p, hi_p = hp_s[0], hp_s[1]
        for c in range(2):
            hr, hi = T[c][:, :B], T[c][:, B:]
            br = sgn * hi
            bi = -sgn * hr
            if not (first and c == 0):
                br = br + hr_p
                bi = bi + hi_p
            g_s[0, 2 * m + c + 1] = br
            g_s[1, 2 * m + c + 1] = bi - br
            g_s[2, 2 * m + c + 1] = br + bi
            hr_p, hi_p = hr, hi
        hp_s[0] = hr_p
        hp_s[1] = hi_p

    def conv_u(m):
        lane = lax.broadcasted_iota(jnp.int32, (RC // 2, B), 1)
        for r in range(D // RC):
            rs = slice(r * RC, (r + 1) * RC)
            if isinstance(m, int) and m == 0:
                halo = jnp.zeros((RC // 2, B), u32)
            else:
                halo = pltpu.bitcast(k_v[m - 1, rs, B:PW], u32)
            tiles = [halo, pltpu.bitcast(k_v[m, rs, 0:B], u32), pltpu.bitcast(k_v[m, rs, B:PW], u32)]
            rolled = [[pltpu.roll(t, j, 1) for t in tiles] for j in range(1, 4)]
            for c in range(2):
                ks = _unpack(tiles[c + 1]).astype(f32) * coef[0, rs]
                for j in range(1, 4):
                    kj = jnp.where(lane >= j, rolled[j - 1][c + 1], rolled[j - 1][c])
                    ks = ks + _unpack(kj).astype(f32) * coef[j, rs]
                kv = (ks * v_v[m, rs, c * B:(c + 1) * B].astype(f32)).astype(bf16)
                y_s[2 * m + c, rs] = kv.astype(f32) * coef[4, rs]
                kv_s[c, r * RC // 2:(r + 1) * RC // 2] = pltpu.bitcast(kv, u32)

    def conv_u_dot(m):
        T = [_dot(_unpack(kv_s[c]), _unpack(ffwd_v[...])) for c in range(2)]
        for c in range(2):
            ar, ai = T[c][:, :B], T[c][:, B:]
            u_s[0, 2 * m + c] = ar + ai
            u_s[1, 2 * m + c] = ar
            u_s[2, 2 * m + c] = ai

    def conv_unit(I, J, init=False):
        dl = 2 * (I - J)
        diag = isinstance(dl, int) and dl == 0
        for r in range(D // UC):
            rs = pl.ds(r * UC, UC)
            k0, k1 = [], []
            for t in range(3):
                gb, gc = g_s[t, dl + 1, rs], g_s[t, dl + 2, rs]
                u0, u1 = u_s[t, 2 * J, rs], u_s[t, 2 * J + 1, rs]
                k0.append(gb * u0 if diag else gb * u0 + g_s[t, dl, rs] * u1)
                k1.append(gc * u0 + gb * u1)
            for a, ks in enumerate((k0, k1)):
                re, im = ks[0] - ks[2], ks[0] + ks[1]
                if init is False:
                    re = ya_s[0, 2 * I + a, rs] + re
                    im = ya_s[1, 2 * I + a, rs] + im
                elif init is not True:
                    re = jnp.where(init, 0.0, ya_s[0, 2 * I + a, rs]) + re
                    im = jnp.where(init, 0.0, ya_s[1, 2 * I + a, rs]) + im
                ya_s[0, 2 * I + a, rs] = re
                ya_s[1, 2 * I + a, rs] = im

    def conv_inverse(m):
        yi = [_dot(jnp.concatenate([ya_s[0, 2 * m + c], ya_s[1, 2 * m + c]], axis=1).astype(bf16),
                   _unpack(finv_v[...])) for c in range(2)]
        for c in range(2):
            y_s[2 * m + c] = y_s[2 * m + c] + yi[c]

    def prep_gu(c, opaque=True):
        c8 = pl.ds(pl.multiple_of(par[10 + c] * 8, 8), 8) if opaque else slice(c * 8, (c + 1) * 8)
        for i, w in enumerate((wg_v, wu_v)):
            wt1 = w[0:KH, c * PW:(c + 1) * PW].T.astype(f32)
            wt2 = w[KH:D, c * PW:(c + 1) * PW].T.astype(f32)
            cs = _acombos(wt1[:B], wt2[:B], wt1[B:], wt2[B:])
            for p in range(7):
                agu[p, c8, i] = _pack(cs[p]).reshape(8, 8, KH)

    def prep_d(chunks):
        for c in chunks:
            w = wd_v[:, c * PW:(c + 1) * PW].astype(f32)
            cs = _acombos(w[:KH, :B], w[:KH, B:], w[KH:, :B], w[KH:, B:])
            for p in range(7):
                ad[p, :, c * B:(c + 1) * B] = _pack(cs[p])

    def item_block(n):
        return 2 * (n // 4) + n % 2

    def head(n, tiles=range(TM // B), chained=True):
        static = isinstance(n, int)
        blk = item_block(n) if static else jnp.minimum(item_block(n), S // TM - 1)
        for c in tiles:
            slot = par[(n % 2) * 4 + c] if chained else n % 2
            rs = slice((c // 2) * D, (c // 2 + 1) * D)
            cs = slice((c % 2) * B, (c % 2 + 1) * B)
            xr = lambda: xb[2 + slot, rs, cs]
            mu = jnp.mean(xr(), axis=0, keepdims=True)
            xc = xr() - mu
            rstd = lax.rsqrt(jnp.mean(xc * xc, axis=0, keepdims=True) + 1e-5)
            x0 = xr()
            x1 = x0 + (x0 - mu) * rstd * y_s[4 * blk + c]
            xb[2 + slot, rs, cs] = x1
            mu = jnp.mean(x1, axis=0, keepdims=True)
            xc = xr() - mu
            rstd = lax.rsqrt(jnp.mean(xc * xc, axis=0, keepdims=True) + 1e-5)
            xb[slot, rs, cs] = (xr() - mu) * rstd

    def load_q(slot, blk, halves=(0, 1)):
        for hf in halves:
            xb[2 + slot, hf * D:(hf + 1) * D] = q_v[2 * blk + hf].astype(f32)

    def b_operand(slot, p):
        b11 = lambda: xb[slot, 0:KH]
        b21 = lambda: xb[slot, KH:D]
        b12 = lambda: xb[slot, D:D + KH]
        b22 = lambda: xb[slot, D + KH:2 * D]
        return (lambda: b11() + b22(), b11, lambda: b12() - b22(), lambda: b21() - b11(), b22,
                lambda: b11() + b12(), lambda: b21() + b22())[p]().astype(bf16)

    def down_and_tail(n, first_item=False):
        slot = n % 2
        blk = item_block(n)

        def Ad(p):
            return _unpack(ad[p])

        def fenced(v):
            top = jnp.where(par[8] == 1, xb[par[9], 0:16], v[0:16])
            return jnp.concatenate([top, v[16:]], axis=0)

        head(par[11] if isinstance(n, int) else n + 1)
        d4 = _dot(Ad(3), (hq[2] - hq[0]).astype(bf16))
        d6 = _dot(Ad(5), (hq[0] + hq[1]).astype(bf16))
        if isinstance(n, int):
            d3 = _dot(Ad(2), (hq[1] - hq[3]).astype(bf16))
            d1 = _dot(Ad(0), (hq[0] + hq[3]).astype(bf16))
            d7 = _dot(Ad(6), (hq[2] + hq[3]).astype(bf16))
            d2 = _dot(Ad(1), fenced(hq[0]).astype(bf16))
            d5 = _dot(Ad(4), hq[3].astype(bf16))
        else:
            d5 = _dot(Ad(4), hq[3].astype(bf16))
            d1 = _dot(Ad(0), (hq[0] + hq[3]).astype(bf16))
            d2 = _dot(Ad(1), fenced(hq[0]).astype(bf16))
            d3 = _dot(Ad(2), (hq[1] - hq[3]).astype(bf16))
            d7 = _dot(Ad(6), (hq[2] + hq[3]).astype(bf16))
        last = (n // 2) % 2 == 1
        for (hf, kh, o) in ((0, 1, d2 + d4), (1, 0, d3 + d5), (1, 1, d1 - d2 + d3 + d6), (0, 0, d1 + d4 - d5 + d7)):
            rs = slice(hf * D + kh * KH, hf * D + (kh + 1) * KH)
            xo = xb[2 + slot, rs] + o
            if isinstance(n, int):
                xb[2 + slot, rs] = xo
            else:
                o_v[blk, kh * KH:(kh + 1) * KH, hf * TH:(hf + 1) * TH] = xo.astype(bf16)
                nb = jnp.minimum(blk + 2, S // TM - 1)
                qn = q_v[2 * nb + hf, kh * KH:(kh + 1) * KH].astype(f32)
                xb[2 + slot, rs] = jnp.where(last, qn, xo)

    wait(in_copies(0) + q_copies((0,)))
    start(gu_copies(1) + gu_copies(2))
    conv_h(0)
    conv_u(0)
    conv_u_dot(0)
    conv_unit(0, 0, init=True)
    conv_inverse(0)
    load_q(0, 0, (0,))
    head(0, (0, 1), False)
    wait(gu_copies(0) + in_copies(1) + q_copies((1,)))
    start(gu_copies(3) + gu_copies(4) + in_copies(2))
    conv_h(1)
    conv_u(1)
    conv_u_dot(1)
    conv_unit(1, 0, init=True)
    conv_unit(1, 1)
    conv_inverse(1)
    prep_gu(0, False)
    load_q(0, 0, (1,))
    head(0, (2, 3), False)
    for p in range(7):
        bc_s[p] = pltpu.bitcast(b_operand(0, p), u32)

    def products(c, hooks=None):
        hooks = hooks or {}
        count = [0]

        def mm(p):
            fence = hooks[count[0]]() if count[0] in hooks else None
            count[0] += 1
            b = bc_s[p]
            if fence is not None:
                b = jnp.concatenate([jnp.where(par[8] == 1, fence, b[0:8]), b[8:]], axis=0)
            return _dot(_unpack(agu[p, c * 8:(c + 1) * 8].reshape(B, KH)), _unpack(b))
        rs = slice(c * B, (c + 1) * B)
        m2, m4 = mm(1), mm(3)
        hq[2, rs] = _act(m2 + m4)
        m5, m3 = mm(4), mm(2)
        hq[1, rs] = _act(m3 + m5)
        m1 = mm(0)
        m7 = mm(6)
        hq[0, rs] = _act(m1 + m4 - m5 + m7)
        m6 = mm(5)
        hq[3, rs] = _act(m1 - m2 + m3 + m6)

    def unit0(s, init=False):
        i = (len(UNITS) * NSLOT + s) * 2
        conv_unit(tab[i], tab[i + 1], init=init)

    def fwd_u(m):
        conv_u(m)
        conv_u_dot(m)

    def units0(lo, hi, inits):
        for s in range(lo, hi):
            unit0(s, s in inits)

    def pd(c):
        def hook():
            prep_d((c,))
            return ad[par[9], 0:8, 0:TH]
        return hook

    wait(gu_copies(1) + gu_copies(2))
    @pl.when(par[8] == 0)
    def _():
        start(gu_copies(5) + gu_copies(6) + in_copies(3) + d_copies() + q_copies((2, 3)))
        products(0)
        prep_gu(1, False)
        products(1, {4: lambda: prep_gu(2)})

    wait(gu_copies(3) + gu_copies(4) + in_copies(2))
    @pl.when(par[8] == 0)
    def _():
        conv_h(par[12])
        products(2, {2: lambda: fwd_u(par[12])})
        prep_gu(3, False)
        units0(0, 4, (0, 3))
        products(3, {4: lambda: prep_gu(4)})
        conv_inverse(par[12])

    wait(gu_copies(5) + gu_copies(6) + in_copies(3) + d_copies() + q_copies((2, 3)))
    @pl.when(par[8] == 0)
    def _():
        start(in_copies(4) + q_copies((4, 5, 6, 7)))
        conv_h(par[13])
        products(4, {2: lambda: fwd_u(par[13])})
        prep_gu(5, False)
        units0(4, 9, (4,))
        products(5)
        prep_gu(6, False)
        load_q(1, 1)
        products(6)
        conv_inverse(par[13])

    @pl.when(par[8] == 0)
    def _():
        prep_d(range(NCH))
        down_and_tail(0)

    def body(n, with_conv):
        slot = n % 2
        m = n + 3

        def unit(s):
            if with_conv:
                i = ((n - 1) * NSLOT + s) * 2
                conv_unit(tab[i], tab[i + 1], init=(n < 4) if s == 0 else False)

        def mm(p):
            return _dot(_unpack(agu[p].reshape(F // 2, KH)), b_operand(slot, p))

        if with_conv:
            wait(in_copies(m))

            @pl.when(m < NP - 1)
            def _():
                start(in_copies(jnp.minimum(m + 1, NP - 1)))
            conv_h(m)
        m2 = mm(1)
        m5 = mm(4)
        if with_conv:
            conv_u(m)
            conv_u_dot(m)
        m1 = mm(0)
        unit(0)
        unit(1)
        m4 = mm(3)
        hq[2] = _act(m2 + m4)
        unit(2)
        m3 = mm(2)
        hq[1] = _act(m3 + m5)
        unit(3)
        unit(4)
        unit(5)
        if with_conv:
            conv_inverse(m)
        m7 = mm(6)
        hq[0] = _act(m1 + m4 - m5 + m7)
        m6 = mm(5)
        hq[3] = _act(m1 - m2 + m3 + m6)
        down_and_tail(n)

        @pl.when((n // 2) % 2 == 1)
        def _():
            out_copy(item_block(n)).start()

    def body_conv(n, carry):
        body(n, True)
        return carry

    def body_plain(n, carry):
        body(n, False)
        return carry

    wait(q_copies((4, 5, 6, 7)))
    lax.fori_loop(1, 5, body_conv, 0)
    lax.fori_loop(5, 8, body_plain, 0)
    for b in range(S // TM):
        out_copy(b).wait()


@jax.jit
def pallas_interleave_layers__ssm_conv_h3__geglu_ffn__prompt_kernel(A_q, A_k, A_v, A_shift_k, A_ssm_k, A_ssm_D, B_x, B_w_gate, B_w_up, B_w_down):
    hbm = pl.BlockSpec(memory_space=pl.ANY)
    out = pl.pallas_call(
        kernel,
        in_specs=[hbm] * 9,
        out_specs=hbm,
        out_shape=jax.ShapeDtypeStruct((D, S), bf16),
        scratch_shapes=[
            pltpu.VMEM((NP, D, PW), bf16), pltpu.VMEM((NP, D, PW), bf16),
            pltpu.VMEM((NP, D, PW), bf16), pltpu.VMEM((NP, D, PW), bf16),
            pltpu.VMEM((D, F), bf16), pltpu.VMEM((D, F), bf16), pltpu.VMEM((D, F), bf16),
            pltpu.VMEM((4, D), bf16), pltpu.VMEM((D,), bf16),
            pltpu.VMEM((7, FH // 16, 2, 8, KH), u32), pltpu.VMEM((7, KH // 2, FH), u32),
            pltpu.VMEM((B // 2, 2 * B), u32), pltpu.VMEM((B, B), u32),
            pltpu.VMEM((5, D, B), f32),
            pltpu.VMEM((3, NB, D, B), f32), pltpu.VMEM((3, NB + 1, D, B), f32),
            pltpu.VMEM((2, D, B), f32), pltpu.VMEM((2, NB, D, B), f32),
            pltpu.VMEM((NB, D, B), f32), pltpu.VMEM((S // TM, D, TM), bf16),
            pltpu.VMEM((2, D // 2, B), u32), pltpu.VMEM((4, FH, TH), f32), pltpu.VMEM((4, FH, TH), f32), pltpu.VMEM((7, KH // 2, TH), u32),
            pltpu.SMEM(((len(UNITS) * NSLOT + len(UNITS0)) * 2,), jnp.int32), pltpu.SMEM((10 + NCH,), jnp.int32),
            pltpu.SemaphoreType.DMA((4 * NP,)), pltpu.SemaphoreType.DMA((2 * NCH + 1,)),
            pltpu.SemaphoreType.DMA((S // TM,)), pltpu.SemaphoreType.DMA((2,)),
        ],
        compiler_params=pltpu.CompilerParams(vmem_limit_bytes=110 * 1024 * 1024),
    )(A_q[0].T, A_k[0].T, A_v[0].T, A_shift_k.T, A_ssm_k, A_ssm_D, B_w_gate, B_w_up, B_w_down.T)
    return out.T[None]
```

```python
import functools
import math
import jax
import jax.numpy as jnp
from jax import lax
from jax.experimental import pallas as pl
from jax.experimental.pallas import tpu as pltpu

S, D, F = 2048, 448, 1792
B = 128
NB = S // B
PW = 2 * B
NP = S // PW
TM = 512
TH = TM // 2
KH = D // 2
FH = F // 2
NCH = F // PW
RC = 32
UC = 16
f32 = jnp.float32
bf16 = jnp.bfloat16
u32 = jnp.uint32

UNITS = (
    ((5, 1), (4, 0), (4, 3), (4, 4), (5, 2), (5, 3)),
    ((6, 1), (5, 0), (5, 4), (5, 5), (6, 2), (6, 3)),
    ((7, 1), (6, 0), (6, 4), (6, 5), (6, 6), (7, 2)),
    ((7, 3), (7, 0), (7, 4), (7, 5), (7, 6), (7, 7)),
)
NSLOT = 6
PADN = 100
MULTI = False
UNITS0 = ((2, 0), (2, 1), (2, 2), (4, 2), (3, 1), (3, 2), (3, 0), (3, 3), (4, 1))


def _dft_mats():
    n = lax.broadcasted_iota(jnp.int32, (B, B), 0)
    f = lax.broadcasted_iota(jnp.int32, (B, B), 1)
    m = ((2 * f + 1) * n) & 511
    m = jnp.where(m >= 256, m - 512, m)
    ang = m.astype(f32) * (math.pi / 256.0)
    ffwd = jnp.concatenate([jnp.cos(ang), -jnp.sin(ang)], axis=1).astype(bf16)
    m2 = ((2 * n + 1) * (f + B)) & 511
    m2 = jnp.where(m2 >= 256, m2 - 512, m2)
    ang2 = m2.astype(f32) * (math.pi / 256.0)
    finv = (jnp.concatenate([jnp.cos(ang2), -jnp.sin(ang2)], axis=0) * (2.0 / 256.0)).astype(bf16)
    return ffwd, finv


def _ln(x):
    m = jnp.mean(x, axis=0, keepdims=True)
    xc = x - m
    v = jnp.mean(xc * xc, axis=0, keepdims=True)
    return xc * lax.rsqrt(v + 1e-5)


def _gelu(x):
    c = math.sqrt(2.0 / math.pi)
    return 0.5 * x * (1.0 + jnp.tanh(c * (x + 0.044715 * (x * x * x))))


def _acombos(a11, a12, a21, a22):
    return [a11 + a22, a21 + a22, a11, a22, a11 + a12, a21 - a11, a12 - a22]


def _pack(x):
    return pltpu.bitcast(x.astype(bf16), u32)


def _unpack(x):
    return pltpu.bitcast(x, bf16)


def _dot(a, b):
    return jnp.dot(a, b, preferred_element_type=f32)


def _act(c):
    rows = c.shape[0] // 2
    c = c.reshape(rows // 16, 2, 16, TH)
    return (_gelu(c[:, 0]) * c[:, 1]).reshape(rows, TH)


def kernel(q_hbm, k_hbm, v_hbm, sk_hbm, h_hbm, d_hbm, wg_hbm, wu_hbm, wd_hbm, o_hbm,
           q_v, k_v, v_v, h_v, wg_v, wu_v, wd_v, sk_v, d_v, agu, ad, ffwd_v, finv_v, coef,
           u_s, g_s, hp_s, ya_s, y_s, o_v, kv_s, hq, xb, bc_s, tab, par, g_sem, in_sem, o_sem):

    def _slab(src, dst, m, sem):
        c0 = m * PW if isinstance(m, int) else pl.multiple_of(m * PW, PW)
        return pltpu.make_async_copy(src.at[:, pl.ds(c0, PW)], dst.at[m], sem)

    def in_copies(m, sem):
        return [_slab(src, dst, m, sem) for src, dst in ((k_hbm, k_v), (v_hbm, v_v), (h_hbm, h_v))]

    def q_copies(ms, sem):
        return [_slab(q_hbm, q_v, m, sem) for m in ms]

    def gu_copies(cs, sem):
        return [pltpu.make_async_copy(src.at[:, pl.ds(c * PW, PW)], dst.at[:, pl.ds(c * PW, PW)], sem)
                for c in cs for src, dst in ((wg_hbm, wg_v), (wu_hbm, wu_v))]

    def group(g):
        sem = g_sem.at[g]
        if g == 0:
            return [pltpu.make_async_copy(sk_hbm, sk_v, sem), pltpu.make_async_copy(d_hbm, d_v, sem)]
        if g == 1:
            return in_copies(0, sem)
        if g == 2:
            return in_copies(1, sem) + q_copies((0,), sem)
        if g == 8:
            return q_copies((1,), sem) + gu_copies((0,), sem)
        if g == 3:
            return gu_copies((1, 2), sem)
        if g == 4:
            return gu_copies((3, 4), sem) + in_copies(2, sem)
        if g == 5:
            return gu_copies((5, 6), sem) + in_copies(3, sem) + q_copies((2, 3), sem)
        if g == 6:
            return [pltpu.make_async_copy(wd_hbm, wd_v, sem)]
        return q_copies((4, 5, 6, 7), sem)

    def late_copies(m):
        return in_copies(m, in_sem.at[m - 4])

    def out_copy(b):
        return pltpu.make_async_copy(o_v.at[b], o_hbm.at[:, pl.ds(b * TM, TM)], o_sem)

    def start(cps):
        for cp in cps:
            cp.start()

    def wait(cps):
        for cp in cps:
            cp.wait()

    start(group(0) + group(1))
    for n in range(len(UNITS)):
        for s in range(NSLOT):
            tab[(n * NSLOT + s) * 2] = UNITS[n][s][0]
            tab[(n * NSLOT + s) * 2 + 1] = UNITS[n][s][1]
    for s, (i, j) in enumerate(UNITS0):
        tab[(len(UNITS) * NSLOT + s) * 2] = i
        tab[(len(UNITS) * NSLOT + s) * 2 + 1] = j

    for i in range(8):
        par[i] = i // 4
    par[8] = 0
    par[9] = 0
    for c in range(NCH):
        par[10 + c] = c
    ffwd, finv = _dft_mats()
    ffwd_v[...] = pltpu.bitcast(ffwd, u32)
    finv_v[...] = pltpu.bitcast(finv, u32)
    zero_blk = jnp.zeros((D, B), f32)
    for t in range(3):
        g_s[t, 0] = zero_blk
    wait(group(0))
    start(group(2))
    sk = sk_v[...].astype(f32)
    dv = d_v[...].astype(f32).reshape(1, D)
    for j in range(5):
        row = sk[j:j + 1] if j < 4 else dv
        coef[j] = jnp.broadcast_to(row, (B, D)).T

    def conv_h(m):
        T = [_dot(h_v[m, :, c * B:(c + 1) * B], _unpack(ffwd_v[...])) for c in range(2)]
        sgn = 1.0 - 2.0 * (lax.broadcasted_iota(jnp.int32, (1, B), 1) & 1).astype(f32)
        first = isinstance(m, int) and m == 0
        if not first:
            hr_p, hi_p = hp_s[0], hp_s[1]
        for c in range(2):
            hr, hi = T[c][:, :B], T[c][:, B:]
            br = sgn * hi
            bi = -sgn * hr
            if not (first and c == 0):
                br = br + hr_p
                bi = bi + hi_p
            g_s[0, 2 * m + c + 1] = br
            g_s[1, 2 * m + c + 1] = bi - br
            g_s[2, 2 * m + c + 1] = br + bi
            hr_p, hi_p = hr, hi
        hp_s[0] = hr_p
        hp_s[1] = hi_p

    def conv_u(m):
        lane = lax.broadcasted_iota(jnp.int32, (RC // 2, B), 1)
        for r in range(D // RC):
            rs = slice(r * RC, (r + 1) * RC)
            if isinstance(m, int) and m == 0:
                halo = jnp.zeros((RC // 2, B), u32)
            else:
                halo = pltpu.bitcast(k_v[m - 1, rs, B:PW], u32)
            tiles = [halo, pltpu.bitcast(k_v[m, rs, 0:B], u32), pltpu.bitcast(k_v[m, rs, B:PW], u32)]
            rolled = [[pltpu.roll(t, j, 1) for t in tiles] for j in range(1, 4)]
            for c in range(2):
                ks = _unpack(tiles[c + 1]).astype(f32) * coef[0, rs]
                for j in range(1, 4):
                    kj = jnp.where(lane >= j, rolled[j - 1][c + 1], rolled[j - 1][c])
                    ks = ks + _unpack(kj).astype(f32) * coef[j, rs]
                kv = (ks * v_v[m, rs, c * B:(c + 1) * B].astype(f32)).astype(bf16)
                y_s[2 * m + c, rs] = kv.astype(f32) * coef[4, rs]
                kv_s[c, r * RC // 2:(r + 1) * RC // 2] = pltpu.bitcast(kv, u32)

    def conv_u_dot(m):
        T = [_dot(_unpack(kv_s[c]), _unpack(ffwd_v[...])) for c in range(2)]
        for c in range(2):
            ar, ai = T[c][:, :B], T[c][:, B:]
            u_s[0, 2 * m + c] = ar + ai
            u_s[1, 2 * m + c] = ar
            u_s[2, 2 * m + c] = ai

    def conv_unit(I, J, init=False):
        dl = 2 * (I - J)
        diag = isinstance(dl, int) and dl == 0
        for r in range(D // UC):
            rs = pl.ds(r * UC, UC)
            k0, k1 = [], []
            for t in range(3):
                gb, gc = g_s[t, dl + 1, rs], g_s[t, dl + 2, rs]
                u0, u1 = u_s[t, 2 * J, rs], u_s[t, 2 * J + 1, rs]
                k0.append(gb * u0 if diag else gb * u0 + g_s[t, dl, rs] * u1)
                k1.append(gc * u0 + gb * u1)
            for a, ks in enumerate((k0, k1)):
                re, im = ks[0] - ks[2], ks[0] + ks[1]
                if init is False:
                    re = ya_s[0, 2 * I + a, rs] + re
                    im = ya_s[1, 2 * I + a, rs] + im
                elif init is not True:
                    re = jnp.where(init, 0.0, ya_s[0, 2 * I + a, rs]) + re
                    im = jnp.where(init, 0.0, ya_s[1, 2 * I + a, rs]) + im
                ya_s[0, 2 * I + a, rs] = re
                ya_s[1, 2 * I + a, rs] = im

    def conv_inverse(m):
        yi = [_dot(jnp.concatenate([ya_s[0, 2 * m + c], ya_s[1, 2 * m + c]], axis=1).astype(bf16),
                   _unpack(finv_v[...])) for c in range(2)]
        for c in range(2):
            y_s[2 * m + c] = y_s[2 * m + c] + yi[c]

    def prep_gu(c, opaque=True):
        c8 = pl.ds(pl.multiple_of(par[10 + c] * 8, 8), 8) if opaque else slice(c * 8, (c + 1) * 8)
        for i, w in enumerate((wg_v, wu_v)):
            wt1 = w[0:KH, c * PW:(c + 1) * PW].T.astype(f32)
            wt2 = w[KH:D, c * PW:(c + 1) * PW].T.astype(f32)
            cs = _acombos(wt1[:B], wt2[:B], wt1[B:], wt2[B:])
            for p in range(7):
                agu[p, c8, i] = _pack(cs[p]).reshape(8, 8, KH)

    def prep_d(chunks):
        for c in chunks:
            w = wd_v[:, c * PW:(c + 1) * PW].astype(f32)
            cs = _acombos(w[:KH, :B], w[:KH, B:], w[KH:, :B], w[KH:, B:])
            for p in range(7):
                ad[p, :, c * B:(c + 1) * B] = _pack(cs[p])

    def item_block(n):
        return 2 * (n // 4) + n % 2

    def head(n, tiles=range(TM // B), chained=True):
        static = isinstance(n, int)
        blk = item_block(n) if static else jnp.minimum(item_block(n), S // TM - 1)
        for c in tiles:
            slot = par[(n % 2) * 4 + c] if chained else n % 2
            rs = slice((c // 2) * D, (c // 2 + 1) * D)
            cs = slice((c % 2) * B, (c % 2 + 1) * B)
            xr = lambda: xb[2 + slot, rs, cs]
            mu = jnp.mean(xr(), axis=0, keepdims=True)
            xc = xr() - mu
            rstd = lax.rsqrt(jnp.mean(xc * xc, axis=0, keepdims=True) + 1e-5)
            x0 = xr()
            x1 = x0 + (x0 - mu) * rstd * y_s[4 * blk + c]
            xb[2 + slot, rs, cs] = x1
            mu = jnp.mean(x1, axis=0, keepdims=True)
            xc = xr() - mu
            rstd = lax.rsqrt(jnp.mean(xc * xc, axis=0, keepdims=True) + 1e-5)
            xb[slot, rs, cs] = (xr() - mu) * rstd

    def load_q(slot, blk, halves=(0, 1)):
        for hf in halves:
            xb[2 + slot, hf * D:(hf + 1) * D] = q_v[2 * blk + hf].astype(f32)

    def b_operand(slot, p):
        b11 = lambda: xb[slot, 0:KH]
        b21 = lambda: xb[slot, KH:D]
        b12 = lambda: xb[slot, D:D + KH]
        b22 = lambda: xb[slot, D + KH:2 * D]
        return (lambda: b11() + b22(), b11, lambda: b12() - b22(), lambda: b21() - b11(), b22,
                lambda: b11() + b12(), lambda: b21() + b22())[p]().astype(bf16)

    def down_and_tail(n, first_item=False):
        slot = n % 2
        blk = item_block(n)

        def Ad(p):
            return _unpack(ad[p])

        def fenced(v):
            top = jnp.where(par[8] == 1, xb[par[9], 0:16], v[0:16])
            return jnp.concatenate([top, v[16:]], axis=0)

        head(par[11] if isinstance(n, int) else n + 1)
        d4 = _dot(Ad(3), (hq[2] - hq[0]).astype(bf16))
        d6 = _dot(Ad(5), (hq[0] + hq[1]).astype(bf16))
        if isinstance(n, int):
            d3 = _dot(Ad(2), (hq[1] - hq[3]).astype(bf16))
            d1 = _dot(Ad(0), (hq[0] + hq[3]).astype(bf16))
            d7 = _dot(Ad(6), (hq[2] + hq[3]).astype(bf16))
            d2 = _dot(Ad(1), fenced(hq[0]).astype(bf16))
            d5 = _dot(Ad(4), hq[3].astype(bf16))
        else:
            d5 = _dot(Ad(4), hq[3].astype(bf16))
            d1 = _dot(Ad(0), (hq[0] + hq[3]).astype(bf16))
            d2 = _dot(Ad(1), fenced(hq[0]).astype(bf16))
            d3 = _dot(Ad(2), (hq[1] - hq[3]).astype(bf16))
            d7 = _dot(Ad(6), (hq[2] + hq[3]).astype(bf16))
        last = (n // 2) % 2 == 1
        for (hf, kh, o) in ((0, 1, d2 + d4), (1, 0, d3 + d5), (1, 1, d1 - d2 + d3 + d6), (0, 0, d1 + d4 - d5 + d7)):
            rs = slice(hf * D + kh * KH, hf * D + (kh + 1) * KH)
            xo = xb[2 + slot, rs] + o
            if isinstance(n, int):
                xb[2 + slot, rs] = xo
            else:
                o_v[blk, kh * KH:(kh + 1) * KH, hf * TH:(hf + 1) * TH] = xo.astype(bf16)
                nb = jnp.minimum(blk + 2, S // TM - 1)
                qn = q_v[2 * nb + hf, kh * KH:(kh + 1) * KH].astype(f32)
                xb[2 + slot, rs] = jnp.where(last, qn, xo)

    wait(group(1))
    start(group(8))
    conv_h(0)
    conv_u(0)
    conv_u_dot(0)
    conv_unit(0, 0, init=True)
    conv_inverse(0)
    wait(group(2))
    start(group(3))
    conv_h(1)
    conv_u(1)
    conv_u_dot(1)
    conv_unit(1, 0, init=True)
    conv_unit(1, 1)
    conv_inverse(1)
    load_q(0, 0, (0,))
    head(0, (0, 1), False)
    wait(group(8))
    start(group(4))
    prep_gu(0, False)
    load_q(0, 0, (1,))
    head(0, (2, 3), False)
    for p in range(7):
        bc_s[p] = pltpu.bitcast(b_operand(0, p), u32)

    def products(c, hooks=None):
        hooks = hooks or {}
        count = [0]

        def mm(p):
            fence = hooks[count[0]]() if count[0] in hooks else None
            count[0] += 1
            b = bc_s[p]
            if fence is not None:
                b = jnp.concatenate([jnp.where(par[8] == 1, fence, b[0:8]), b[8:]], axis=0)
            return _dot(_unpack(agu[p, c * 8:(c + 1) * 8].reshape(B, KH)), _unpack(b))
        rs = slice(c * B, (c + 1) * B)
        m2, m4 = mm(1), mm(3)
        hq[2, rs] = _act(m2 + m4)
        m5, m3 = mm(4), mm(2)
        hq[1, rs] = _act(m3 + m5)
        m1 = mm(0)
        m7 = mm(6)
        hq[0, rs] = _act(m1 + m4 - m5 + m7)
        m6 = mm(5)
        hq[3, rs] = _act(m1 - m2 + m3 + m6)

    def unit0(s, init=False):
        i = (len(UNITS) * NSLOT + s) * 2
        conv_unit(tab[i], tab[i + 1], init=init)

    def fwd_u(m):
        conv_u(m)
        conv_u_dot(m)

    def units0(lo, hi, inits):
        for s in range(lo, hi):
            unit0(s, s in inits)

    def pd(c):
        def hook():
            prep_d((c,))
            return ad[par[9], 0:8, 0:TH]
        return hook

    wait(group(3))
    @pl.when(par[8] == 0)
    def _():
        start(group(5) + group(6))
        products(0)
        prep_gu(1, False)
        products(1, {4: lambda: prep_gu(2)})

    wait(group(4))
    @pl.when(par[8] == 0)
    def _():
        conv_h(par[12])
        products(2, {2: lambda: fwd_u(par[12])})
        prep_gu(3, False)
        units0(0, 4, (0, 3))
        products(3, {4: lambda: prep_gu(4)})
        conv_inverse(par[12])

    wait(group(5))
    @pl.when(par[8] == 0)
    def _():
        start(late_copies(4) + group(7))
        conv_h(par[13])
        products(4, {2: lambda: fwd_u(par[13])})
        prep_gu(5, False)
        units0(4, 9, (4,))
        products(5)
        prep_gu(6, False)
        load_q(1, 1)
        products(6)
        conv_inverse(par[13])

    wait(group(6))
    @pl.when(par[8] == 0)
    def _():
        prep_d(range(NCH))
        down_and_tail(0)

    def body(n, with_conv):
        slot = n % 2
        m = n + 3

        def unit(s):
            if with_conv:
                i = ((n - 1) * NSLOT + s) * 2
                conv_unit(tab[i], tab[i + 1], init=(n < 4) if s == 0 else False)

        def mm(p):
            return _dot(_unpack(agu[p].reshape(F // 2, KH)), b_operand(slot, p))

        if with_conv:
            wait(late_copies(m))
            conv_h(m)
        m2 = mm(1)
        m5 = mm(4)
        if with_conv:
            conv_u(m)
            conv_u_dot(m)
        m1 = mm(0)
        unit(0)
        unit(1)
        m4 = mm(3)
        hq[2] = _act(m2 + m4)
        unit(2)
        m3 = mm(2)
        hq[1] = _act(m3 + m5)
        unit(3)
        unit(4)
        unit(5)
        if with_conv:
            conv_inverse(m)
        m7 = mm(6)
        hq[0] = _act(m1 + m4 - m5 + m7)
        m6 = mm(5)
        hq[3] = _act(m1 - m2 + m3 + m6)
        down_and_tail(n)

        @pl.when((n // 2) % 2 == 1)
        def _():
            out_copy(item_block(n)).start()

    def body_conv(n, carry):
        body(n, True)
        return carry

    def body_plain(n, carry):
        body(n, False)
        return carry

    wait(group(7))
    start(late_copies(5) + late_copies(6) + late_copies(7))
    lax.fori_loop(1, 5, body_conv, 0)
    lax.fori_loop(5, 8, body_plain, 0)
    for b in range(S // TM):
        out_copy(b).wait()


@jax.jit
def pallas_interleave_layers__ssm_conv_h3__geglu_ffn__prompt_kernel(A_q, A_k, A_v, A_shift_k, A_ssm_k, A_ssm_D, B_x, B_w_gate, B_w_up, B_w_down):
    hbm = pl.BlockSpec(memory_space=pl.ANY)
    out = pl.pallas_call(
        kernel,
        in_specs=[hbm] * 9,
        out_specs=hbm,
        out_shape=jax.ShapeDtypeStruct((D, S), bf16),
        scratch_shapes=[
            pltpu.VMEM((NP, D, PW), bf16), pltpu.VMEM((NP, D, PW), bf16),
            pltpu.VMEM((NP, D, PW), bf16), pltpu.VMEM((NP, D, PW), bf16),
            pltpu.VMEM((D, F), bf16), pltpu.VMEM((D, F), bf16), pltpu.VMEM((D, F), bf16),
            pltpu.VMEM((4, D), bf16), pltpu.VMEM((D,), bf16),
            pltpu.VMEM((7, FH // 16, 2, 8, KH), u32), pltpu.VMEM((7, KH // 2, FH), u32),
            pltpu.VMEM((B // 2, 2 * B), u32), pltpu.VMEM((B, B), u32),
            pltpu.VMEM((5, D, B), f32),
            pltpu.VMEM((3, NB, D, B), f32), pltpu.VMEM((3, NB + 1, D, B), f32),
            pltpu.VMEM((2, D, B), f32), pltpu.VMEM((2, NB, D, B), f32),
            pltpu.VMEM((NB, D, B), f32), pltpu.VMEM((S // TM, D, TM), bf16),
            pltpu.VMEM((2, D // 2, B), u32), pltpu.VMEM((4, FH, TH), f32), pltpu.VMEM((4, FH, TH), f32), pltpu.VMEM((7, KH // 2, TH), u32),
            pltpu.SMEM(((len(UNITS) * NSLOT + len(UNITS0)) * 2,), jnp.int32), pltpu.SMEM((10 + NCH,), jnp.int32),
            pltpu.SemaphoreType.DMA((9,)), pltpu.SemaphoreType.DMA((4,)), pltpu.SemaphoreType.DMA(()),
        ],
        compiler_params=pltpu.CompilerParams(vmem_limit_bytes=110 * 1024 * 1024),
    )(A_q[0].T, A_k[0].T, A_v[0].T, A_shift_k.T, A_ssm_k, A_ssm_D, B_w_gate, B_w_up, B_w_down.T)
    return out.T[None]
```

```python
import math

import jax
import jax.numpy as jnp
from jax import lax
from jax.experimental import pallas as pl
from jax.experimental.pallas import tpu as pltpu

S, D, F = 2048, 448, 1792
B = 128
NB = S // B
PW = 2 * B
NP = S // PW
TM = 512
TH = TM // 2
NT = S // TM
KH = D // 2
FH = F // 2
NCH = F // PW
RC = 32
UC = 32
EPS = 1e-5
f32 = jnp.float32
bf16 = jnp.bfloat16
u32 = jnp.uint32

UNITS = (
    ((5, 1), (4, 0), (4, 3), (4, 4), (5, 2), (5, 3)),
    ((6, 1), (5, 0), (5, 4), (5, 5), (6, 2), (6, 3)),
    ((7, 1), (6, 0), (6, 4), (6, 5), (6, 6), (7, 2)),
    ((7, 3), (7, 0), (7, 4), (7, 5), (7, 6), (7, 7)),
)
NSLOT = 6
UNITS0 = ((2, 0), (2, 1), (2, 2), (4, 2), (3, 1), (3, 2), (3, 0), (3, 3), (4, 1))
P_ZERO, P_ZERO2, P_INT = 8, 9, 10


def _angle(m):
    m = m & 511
    m = jnp.where(m >= 256, m - 512, m)
    return m.astype(f32) * (math.pi / 256.0)


def _dft_mats():
    r = lax.broadcasted_iota(jnp.int32, (B, B), 0)
    c = lax.broadcasted_iota(jnp.int32, (B, B), 1)
    ang = _angle((2 * c + 1) * r)
    ffwd = jnp.concatenate([jnp.cos(ang), -jnp.sin(ang)], axis=1).astype(bf16)
    ang = _angle((2 * r + 1) * (c + B))
    finv = (jnp.concatenate([jnp.cos(ang), -jnp.sin(ang)], axis=0) * (2.0 / 256.0)).astype(bf16)
    return ffwd, finv


def _gelu(x):
    c = math.sqrt(2.0 / math.pi)
    return 0.5 * x * (1.0 + jnp.tanh(c * (x + 0.044715 * (x * x * x))))


def _acombos(a11, a12, a21, a22):
    return [a11 + a22, a21 + a22, a11, a22, a11 + a12, a21 - a11, a12 - a22]


def _bcombos(b11, b12, b21, b22):
    return [b11 + b22, b11, b12 - b22, b21 - b11, b22, b11 + b12, b21 + b22]


def _split(w):
    return pltpu.bitcast(w << 16, f32), pltpu.bitcast(w & jnp.uint32(0xFFFF0000), f32)


def _join(lo, hi):
    return pltpu.pack_elementwise([lo, hi], packed_dtype=bf16).astype(u32)


def _acombos_packed(w11, w12, w21, w22):
    parts = [_split(w) for w in (w11, w12, w21, w22)]
    lo = _acombos(*[p[0] for p in parts])
    hi = _acombos(*[p[1] for p in parts])
    out = [_join(a, b) for a, b in zip(lo, hi)]
    out[2] = w11
    out[3] = w22
    return out


def _words(x):
    return pltpu.bitcast(x, u32)


def _halves(x):
    return pltpu.bitcast(x, bf16)


def _dot(a, b):
    return jnp.dot(a, b, preferred_element_type=f32)


def _act(c):
    rows = c.shape[0] // 2
    c = c.reshape(rows // 16, 2, 16, TH)
    return (_gelu(c[:, 0]) * c[:, 1]).reshape(rows, TH)


def _kernel(q_hbm, k_hbm, v_hbm, sk_hbm, h_hbm, d_hbm, wg_hbm, wu_hbm, wd_hbm, o_hbm,
            q_v, k_v, v_v, h_v, wg_v, wu_v, wd_v, sk_v, d_v, agu, ad, ffwd_v, finv_v, coef,
            u_s, g_s, hp_s, ya_s, y_s, o_v, kv_s, hq, xb, bc_s, xt, tab, par, g_sem, in_sem, o_sem):

    def slab(src, dst, m, sem):
        c0 = m * PW if isinstance(m, int) else pl.multiple_of(m * PW, PW)
        return pltpu.make_async_copy(src.at[:, pl.ds(c0, PW)], dst.at[m], sem)

    def in_copies(m, sem):
        return [slab(src, dst, m, sem) for src, dst in ((k_hbm, k_v), (v_hbm, v_v), (h_hbm, h_v))]

    def q_copies(ms, sem):
        return [slab(q_hbm, q_v, m, sem) for m in ms]

    def gu_copies(cs, sem):
        return [pltpu.make_async_copy(src.at[:, pl.ds(c * PW, PW)], dst.at[:, pl.ds(c * PW, PW)], sem)
                for c in cs for src, dst in ((wg_hbm, wg_v), (wu_hbm, wu_v))]

    def group(g):
        sem = g_sem.at[g]
        if g == 0:
            return [pltpu.make_async_copy(sk_hbm, sk_v, sem), pltpu.make_async_copy(d_hbm, d_v, sem)]
        if g == 1:
            return in_copies(0, sem)
        if g == 2:
            return in_copies(1, sem)
        if g == 8:
            return q_copies((0, 1), sem) + gu_copies((0,), sem)
        if g == 3:
            return gu_copies((1, 2), sem)
        if g == 4:
            return gu_copies((3, 4), sem) + in_copies(2, sem)
        if g == 5:
            return gu_copies((5, 6), sem) + in_copies(3, sem) + q_copies((2, 3), sem)
        if g == 6:
            return [pltpu.make_async_copy(wd_hbm, wd_v, sem)]
        return q_copies((4, 5, 6, 7), sem)

    def late_copies(m):
        return in_copies(m, in_sem.at[m - 4])

    def out_copy(b, slot):
        return pltpu.make_async_copy(o_v.at[b], o_hbm.at[:, pl.ds(b * TM, TM)], o_sem.at[slot])

    def out_quadrant(b, slot, hf, kh):
        c0 = pl.multiple_of(b * TM + hf * TH, TH)
        return pltpu.make_async_copy(o_v.at[b, pl.ds(kh * KH, KH), pl.ds(hf * TH, TH)],
                                     o_hbm.at[pl.ds(kh * KH, KH), pl.ds(c0, TH)], o_sem.at[slot])

    def start(cps):
        for cp in cps:
            cp.start()

    def wait(cps):
        for cp in cps:
            cp.wait()

    def conv_h(m):
        spec = [_dot(h_v[m, :, c * B:(c + 1) * B], _halves(ffwd_v[...])) for c in range(2)]
        sgn = 1.0 - 2.0 * (lax.broadcasted_iota(jnp.int32, (1, B), 1) & 1).astype(f32)
        first = isinstance(m, int) and m == 0
        if not first:
            hr_p, hi_p = hp_s[0], hp_s[1]
        for c in range(2):
            hr, hi = spec[c][:, :B], spec[c][:, B:]
            br = sgn * hi
            bi = -sgn * hr
            if not (first and c == 0):
                br = br + hr_p
                bi = bi + hi_p
            g_s[0, 2 * m + c + 1] = br
            g_s[1, 2 * m + c + 1] = bi - br
            g_s[2, 2 * m + c + 1] = br + bi
            hr_p, hi_p = hr, hi
        hp_s[0] = hr_p
        hp_s[1] = hi_p

    def conv_u(m):
        lane = lax.broadcasted_iota(jnp.int32, (RC // 2, B), 1)
        for r in range(D // RC):
            rs = slice(r * RC, (r + 1) * RC)
            if isinstance(m, int) and m == 0:
                halo = jnp.zeros((RC // 2, B), u32)
            else:
                halo = _words(k_v[m - 1, rs, B:PW])
            tiles = [halo, _words(k_v[m, rs, 0:B]), _words(k_v[m, rs, B:PW])]
            rolled = [[pltpu.roll(t, j, 1) for t in tiles] for j in range(1, 4)]
            cf = [[coef[j, pl.ds(r * RC + e, RC // 2, stride=2)] for e in range(2)] for j in range(4)]
            for c in range(2):
                ks = None
                for j in range(4):
                    kj = tiles[c + 1] if j == 0 else jnp.where(lane >= j, rolled[j - 1][c + 1], rolled[j - 1][c])
                    t = [a * b for a, b in zip(_split(kj), cf[j])]
                    ks = t if ks is None else [a + b for a, b in zip(ks, t)]
                vs = _split(_words(v_v[m, rs, c * B:(c + 1) * B]))
                kv = _join(ks[0] * vs[0], ks[1] * vs[1])
                y_s[2 * m + c, rs] = _halves(kv).astype(f32) * coef[4, rs]
                kv_s[c, r * RC // 2:(r + 1) * RC // 2] = kv
        spec = [_dot(_halves(kv_s[c]), _halves(ffwd_v[...])) for c in range(2)]
        for c in range(2):
            ar, ai = spec[c][:, :B], spec[c][:, B:]
            u_s[0, 2 * m + c] = ar + ai
            u_s[1, 2 * m + c] = ar
            u_s[2, 2 * m + c] = ai

    def conv_unit(i_out, j_in, init=False):
        dl = 2 * (i_out - j_in)
        diag = isinstance(dl, int) and dl == 0
        for r in range(D // UC):
            rs = pl.ds(r * UC, UC)
            k0, k1 = [], []
            for t in range(3):
                gb, gc = g_s[t, dl + 1, rs], g_s[t, dl + 2, rs]
                u0, u1 = u_s[t, 2 * j_in, rs], u_s[t, 2 * j_in + 1, rs]
                k0.append(gb * u0 if diag else gb * u0 + g_s[t, dl, rs] * u1)
                k1.append(gc * u0 + gb * u1)
            for a, ks in enumerate((k0, k1)):
                re, im = ks[0] - ks[2], ks[0] + ks[1]
                if init is False:
                    re = ya_s[0, 2 * i_out + a, rs] + re
                    im = ya_s[1, 2 * i_out + a, rs] + im
                elif init is not True:
                    re = jnp.where(init, 0.0, ya_s[0, 2 * i_out + a, rs]) + re
                    im = jnp.where(init, 0.0, ya_s[1, 2 * i_out + a, rs]) + im
                ya_s[0, 2 * i_out + a, rs] = re
                ya_s[1, 2 * i_out + a, rs] = im

    def table_unit(s, init=False):
        conv_unit(tab[2 * s], tab[2 * s + 1], init=init)

    def conv_inverse(m):
        yi = [_dot(jnp.concatenate([ya_s[0, 2 * m + c], ya_s[1, 2 * m + c]], axis=1).astype(bf16),
                   _halves(finv_v[...])) for c in range(2)]
        for c in range(2):
            y_s[2 * m + c] = y_s[2 * m + c] + yi[c]

    def prep_gu(c, from_table=False):
        c8 = pl.ds(pl.multiple_of(par[P_INT + c] * 8, 8), 8) if from_table else slice(c * 8, (c + 1) * 8)
        hb = B // 2
        for i, w in enumerate((wg_v, wu_v)):
            wt1 = _words(w[0:KH, c * PW:(c + 1) * PW].T)
            wt2 = _words(w[KH:D, c * PW:(c + 1) * PW].T)
            cs = _acombos_packed(wt1[:hb], wt2[:hb], wt1[hb:], wt2[hb:])
            for p in range(7):
                agu[p, c8, i] = cs[p].reshape(8, 8, KH)

    def prep_d():
        hk = KH // 2
        for c in range(NCH):
            w = _words(wd_v[:, c * PW:(c + 1) * PW])
            cs = _acombos_packed(w[:hk, :B], w[:hk, B:], w[hk:, :B], w[hk:, B:])
            for p in range(7):
                ad[p, :, c * B:(c + 1) * B] = cs[p]

    def item_block(n):
        return 2 * (n // 4) + n % 2

    def head(n):
        static = isinstance(n, int)
        blk = item_block(n) if static else jnp.minimum(item_block(n), NT - 1)
        for c in range(TM // B):
            slot = n % 2 if static else par[(n % 2) * 4 + c]
            rs = slice((c // 2) * D, (c // 2 + 1) * D)
            cs = slice((c % 2) * B, (c % 2 + 1) * B)
            xr = lambda: xb[2 + slot, rs, cs]
            mu = jnp.mean(xr(), axis=0, keepdims=True)
            xc = xr() - mu
            rstd = lax.rsqrt(jnp.mean(xc * xc, axis=0, keepdims=True) + EPS)
            x0 = xr()
            x1 = x0 + (x0 - mu) * rstd * y_s[4 * blk + c]
            xb[2 + slot, rs, cs] = x1
            mu = jnp.mean(x1, axis=0, keepdims=True)
            xc = xr() - mu
            rstd = lax.rsqrt(jnp.mean(xc * xc, axis=0, keepdims=True) + EPS)
            if static:
                xt[c, 0:D] = (xr() - mu) * rstd
            else:
                xb[slot, rs, cs] = (xr() - mu) * rstd

    def load_q(slot, blk):
        for hf in range(2):
            xb[2 + slot, hf * D:(hf + 1) * D] = q_v[2 * blk + hf].astype(f32)

    def b_operand(slot, p):
        b11 = lambda: xb[slot, 0:KH]
        b21 = lambda: xb[slot, KH:D]
        b12 = lambda: xb[slot, D:D + KH]
        b22 = lambda: xb[slot, D + KH:2 * D]
        return (lambda: b11() + b22(), b11, lambda: b12() - b22(), lambda: b21() - b11(), b22,
                lambda: b11() + b12(), lambda: b21() + b22())[p]().astype(bf16)

    def down_and_tail(n, fence_at=2, eager_out=False):
        static = isinstance(n, int)
        slot = n % 2
        blk = item_block(n)

        def down(k, p, v):
            if k == fence_at:
                top = jnp.where(par[P_ZERO] == 1, xb[par[P_ZERO2], 0:16], v[0:16])
                v = jnp.concatenate([top, v[16:]], axis=0)
            return _dot(_halves(ad[p]), v.astype(bf16))

        head(par[P_INT + 1] if static else n + 1)
        d4 = down(4, 3, hq[2] - hq[0])
        d6 = down(6, 5, hq[0] + hq[1])
        if static:
            d3 = down(3, 2, hq[1] - hq[3])
            d1 = down(1, 0, hq[0] + hq[3])
            d7 = down(7, 6, hq[2] + hq[3])
            d2 = down(2, 1, hq[0])
            d5 = down(5, 4, hq[3])
        else:
            d5 = down(5, 4, hq[3])
            d1 = down(1, 0, hq[0] + hq[3])
            d2 = down(2, 1, hq[0])
            d3 = down(3, 2, hq[1] - hq[3])
            d7 = down(7, 6, hq[2] + hq[3])
        last = (n // 2) % 2 == 1
        for hf, kh, o in ((0, 1, d2 + d4), (1, 0, d3 + d5), (1, 1, d1 - d2 + d3 + d6), (0, 0, d1 + d4 - d5 + d7)):
            rs = slice(hf * D + kh * KH, hf * D + (kh + 1) * KH)
            xo = xb[2 + slot, rs] + o
            if static:
                xb[2 + slot, rs] = xo
            else:
                o_v[blk, kh * KH:(kh + 1) * KH, hf * TH:(hf + 1) * TH] = xo.astype(bf16)
                if eager_out:
                    out_quadrant(blk, slot, hf, kh).start()
                nb = jnp.minimum(blk + 2, NT - 1)
                qn = q_v[2 * nb + hf, kh * KH:(kh + 1) * KH].astype(f32)
                xb[2 + slot, rs] = jnp.where(last, qn, xo)

    def products(c, hooks=None):
        hooks = hooks or {}
        count = [0]

        def mm(p):
            if count[0] in hooks:
                hooks[count[0]]()
            count[0] += 1
            return _dot(_halves(agu[p, c * 8:(c + 1) * 8].reshape(B, KH)), _halves(bc_s[p]))

        rs = slice(c * B, (c + 1) * B)
        m2, m4 = mm(1), mm(3)
        hq[2, rs] = _act(m2 + m4)
        m5, m3 = mm(4), mm(2)
        hq[1, rs] = _act(m3 + m5)
        m1 = mm(0)
        m7 = mm(6)
        hq[0, rs] = _act(m1 + m4 - m5 + m7)
        m6 = mm(5)
        hq[3, rs] = _act(m1 - m2 + m3 + m6)

    def units0(lo, hi, inits):
        for s in range(lo, hi):
            table_unit(len(UNITS) * NSLOT + s, s in inits)

    def block(fn):
        pl.when(par[P_ZERO] == 0)(fn)

    start(group(0) + group(1))
    for s, (i, j) in enumerate([u for row in UNITS for u in row] + list(UNITS0)):
        tab[2 * s] = i
        tab[2 * s + 1] = j
    for i in range(8):
        par[i] = i // 4
    par[P_ZERO] = 0
    par[P_ZERO2] = 0
    for c in range(NCH):
        par[P_INT + c] = c
    ffwd, finv = _dft_mats()
    ffwd_v[...] = _words(ffwd)
    finv_v[...] = _words(finv)
    for t in range(3):
        g_s[t, 0] = jnp.zeros((D, B), f32)
    wait(group(0))
    start(group(2))
    sk = sk_v[...].astype(f32)
    dv = d_v[...].astype(f32).reshape(1, D)
    for j in range(5):
        row = sk[j:j + 1] if j < 4 else dv
        coef[j, 0:D] = jnp.broadcast_to(row, (B, D)).T

    wait(group(1))
    start(group(8))
    conv_h(0)
    conv_u(0)
    conv_unit(0, 0, init=True)
    conv_inverse(0)
    wait(group(2))
    start(group(3))
    conv_h(1)
    conv_u(1)
    conv_unit(1, 0, init=True)
    conv_unit(1, 1)
    conv_inverse(1)
    wait(group(8))
    start(group(4))
    prep_gu(0)
    load_q(0, 0)
    head(0)
    for cc in range(2):
        def quad(kh, hf, e):
            return xt[2 * hf + cc, pl.ds(kh * KH + e, KH // 2, stride=2)]
        parts = [_bcombos(quad(0, 0, e), quad(0, 1, e), quad(1, 0, e), quad(1, 1, e)) for e in range(2)]
        for p in range(7):
            bc_s[p, :, cc * B:(cc + 1) * B] = _join(parts[0][p], parts[1][p])
    xb[0, 0:16] = jnp.zeros((16, TH), f32)

    wait(group(3))
    start(group(5) + group(6))

    @block
    def _():
        products(0)
        prep_gu(1)
        products(1, {1: lambda: prep_gu(2, True)})

    wait(group(4))

    @block
    def _():
        m = par[P_INT + 2]
        products(2, {1: lambda: conv_h(m), 3: lambda: conv_u(m)})
        prep_gu(3)
        units0(0, 4, (0, 3))
        products(3)
        conv_inverse(m)
        prep_gu(4)

    wait(group(5))
    start(late_copies(4) + group(7))

    @block
    def _():
        m = par[P_INT + 3]
        products(4, {1: lambda: conv_h(m), 3: lambda: conv_u(m)})
        prep_gu(5)
        units0(4, 9, (4,))
        products(5)
        prep_gu(6)
        load_q(1, 1)
        products(6)
        conv_inverse(m)

    wait(group(6))

    @block
    def _():
        prep_d()
        down_and_tail(0)

    def body(n, with_conv):
        slot = n % 2
        m = n + 3

        def unit(s):
            if with_conv:
                table_unit((n - 1) * NSLOT + s, (n < 4) if s == 0 else False)

        def mm(p):
            return _dot(_halves(agu[p].reshape(F // 2, KH)), b_operand(slot, p))

        if with_conv:
            wait(late_copies(m))
            conv_h(m)
        else:
            out_copy(0, slot).wait()
        m2 = mm(1)
        if with_conv:
            conv_u(m)
        m5 = mm(4)
        unit(0)
        unit(1)
        m1 = mm(0)
        unit(2)
        unit(3)
        m4 = mm(3)
        hq[2] = _act(m2 + m4)
        unit(4)
        unit(5)
        m3 = mm(2)
        hq[1] = _act(m3 + m5)
        if with_conv:
            conv_inverse(m)
        m7 = mm(6)
        hq[0] = _act(m1 + m4 - m5 + m7)
        m6 = mm(5)
        hq[3] = _act(m1 - m2 + m3 + m6)
        down_and_tail(n, 2 if with_conv else 5, not with_conv)

        if with_conv:
            @pl.when((n // 2) % 2 == 1)
            def _():
                out_copy(item_block(n), slot).start()

    def body_conv(n, carry):
        body(n, True)
        return carry

    def body_plain(n, carry):
        body(n, False)
        return carry

    wait(group(7))
    start(late_copies(5) + late_copies(6) + late_copies(7))
    lax.fori_loop(1, 5, body_conv, 0)
    lax.fori_loop(5, 8, body_plain, 0)
    for slot in range(2):
        out_copy(0, slot).wait()


@jax.jit
def pallas_interleave_layers__ssm_conv_h3__geglu_ffn__prompt_kernel(A_q, A_k, A_v, A_shift_k, A_ssm_k, A_ssm_D, B_x, B_w_gate, B_w_up, B_w_down):
    hbm = pl.BlockSpec(memory_space=pl.ANY)
    out = pl.pallas_call(
        _kernel,
        in_specs=[hbm] * 9,
        out_specs=hbm,
        out_shape=jax.ShapeDtypeStruct((D, S), bf16),
        scratch_shapes=[
            pltpu.VMEM((NP, D, PW), bf16),
            pltpu.VMEM((NP, D, PW), bf16),
            pltpu.VMEM((NP, D, PW), bf16),
            pltpu.VMEM((NP, D, PW), bf16),
            pltpu.VMEM((D, F), bf16),
            pltpu.VMEM((D, F), bf16),
            pltpu.VMEM((D, F), bf16),
            pltpu.VMEM((4, D), bf16),
            pltpu.VMEM((D,), bf16),
            pltpu.VMEM((7, FH // 16, 2, 8, KH), u32),
            pltpu.VMEM((7, KH // 2, FH), u32),
            pltpu.VMEM((B // 2, 2 * B), u32),
            pltpu.VMEM((B, B), u32),
            pltpu.VMEM((5, D + 8, B), f32),
            pltpu.VMEM((3, NB, D, B), f32),
            pltpu.VMEM((3, NB + 1, D, B), f32),
            pltpu.VMEM((2, D, B), f32),
            pltpu.VMEM((2, NB, D, B), f32),
            pltpu.VMEM((NB, D, B), f32),
            pltpu.VMEM((NT, D, TM), bf16),
            pltpu.VMEM((2, D // 2, B), u32),
            pltpu.VMEM((4, FH, TH), f32),
            pltpu.VMEM((4, FH, TH), f32),
            pltpu.VMEM((7, KH // 2, TH), u32),
            pltpu.VMEM((TM // B, D + 8, B), f32),
            pltpu.SMEM((2 * (len(UNITS) * NSLOT + len(UNITS0)),), jnp.int32),
            pltpu.SMEM((P_INT + NCH,), jnp.int32),
            pltpu.SemaphoreType.DMA((9,)),
            pltpu.SemaphoreType.DMA((4,)),
            pltpu.SemaphoreType.DMA((2,)),
        ],
        compiler_params=pltpu.CompilerParams(vmem_limit_bytes=110 * 1024 * 1024),
    )(A_q[0].T, A_k[0].T, A_v[0].T, A_shift_k.T, A_ssm_k, A_ssm_D, B_w_gate, B_w_up, B_w_down.T)
    return out.T[None]
```

```python
import math

import jax
import jax.numpy as jnp
from jax import lax
from jax.experimental import pallas as pl
from jax.experimental.pallas import tpu as pltpu

S, D, F = 2048, 448, 1792
B = 128
NB = S // B
PW = 2 * B
NP = S // PW
TM = 512
TH = TM // 2
NT = S // TM
KH = D // 2
FH = F // 2
NCH = F // PW
RC = 32
UC = 32
EPS = 1e-5
f32 = jnp.float32
bf16 = jnp.bfloat16
u32 = jnp.uint32

UNITS = (
    ((5, 1), (4, 0), (4, 3), (4, 4), (5, 2), (5, 3)),
    ((6, 1), (5, 0), (5, 4), (5, 5), (6, 2), (6, 3)),
    ((7, 1), (6, 0), (6, 4), (6, 5), (6, 6), (7, 2)),
    ((7, 3), (7, 0), (7, 4), (7, 5), (7, 6), (7, 7)),
)
NSLOT = 6
UNITS0 = ((2, 0), (2, 1), (2, 2), (4, 2), (3, 1), (3, 2), (3, 0), (3, 3), (4, 1))
P_ZERO, P_ZERO2, P_INT = 8, 9, 10
NSTAGE = 40


def _angle(m):
    m = m & 511
    m = jnp.where(m >= 256, m - 512, m)
    return m.astype(f32) * (math.pi / 256.0)


def _dft_mats():
    r = lax.broadcasted_iota(jnp.int32, (B, B), 0)
    c = lax.broadcasted_iota(jnp.int32, (B, B), 1)
    ang = _angle((2 * c + 1) * r)
    ffwd = jnp.concatenate([jnp.cos(ang), -jnp.sin(ang)], axis=1).astype(bf16)
    ang = _angle((2 * r + 1) * (c + B))
    finv = (jnp.concatenate([jnp.cos(ang), -jnp.sin(ang)], axis=0) * (2.0 / 256.0)).astype(bf16)
    return ffwd, finv


def _gelu(x):
    c = math.sqrt(2.0 / math.pi)
    return 0.5 * x * (1.0 + jnp.tanh(c * (x + 0.044715 * (x * x * x))))


def _acombos(a11, a12, a21, a22):
    return [a11 + a22, a21 + a22, a11, a22, a11 + a12, a21 - a11, a12 - a22]


def _bcombos(b11, b12, b21, b22):
    return [b11 + b22, b11, b12 - b22, b21 - b11, b22, b11 + b12, b21 + b22]


def _words(x):
    return pltpu.bitcast(x, u32)


def _halves(x):
    return pltpu.bitcast(x, bf16)


def _dot(a, b):
    return jnp.dot(a, b, preferred_element_type=f32)


def _act(c):
    rows = c.shape[0] // 2
    c = c.reshape(rows // 16, 2, 16, TH)
    return (_gelu(c[:, 0]) * c[:, 1]).reshape(rows, TH)


def _kernel(q_hbm, k_hbm, v_hbm, sk_hbm, h_hbm, d_hbm, wg_hbm, wu_hbm, wd_hbm, o_hbm,
            q_v, k_v, v_v, h_v, wg_v, wu_v, wd_v, sk_v, d_v, agu, ad, ffwd_v, finv_v, coef,
            u_s, g_s, hp_s, ya_s, y_s, o_v, kv_s, hq, xb, bc_s, stage, tab, par, g_sem, in_sem, o_sem):

    def slab(src, dst, m, sem):
        c0 = m * PW if isinstance(m, int) else pl.multiple_of(m * PW, PW)
        return pltpu.make_async_copy(src.at[:, pl.ds(c0, PW)], dst.at[m], sem)

    def in_copies(m, sem):
        return [slab(src, dst, m, sem) for src, dst in ((k_hbm, k_v), (v_hbm, v_v), (h_hbm, h_v))]

    def q_copies(ms, sem):
        return [slab(q_hbm, q_v, m, sem) for m in ms]

    def gu_copies(cs, sem):
        return [pltpu.make_async_copy(src.at[:, pl.ds(c * PW, PW)], dst.at[:, pl.ds(c * PW, PW)], sem)
                for c in cs for src, dst in ((wg_hbm, wg_v), (wu_hbm, wu_v))]

    def group(g):
        sem = g_sem.at[g]
        if g == 0:
            return [pltpu.make_async_copy(sk_hbm, sk_v, sem), pltpu.make_async_copy(d_hbm, d_v, sem)]
        if g == 1:
            return in_copies(0, sem)
        if g == 2:
            return in_copies(1, sem)
        if g == 8:
            return q_copies((0, 1), sem) + gu_copies((0,), sem)
        if g == 3:
            return gu_copies((1, 2), sem)
        if g == 4:
            return gu_copies((3, 4), sem) + in_copies(2, sem)
        if g == 5:
            return gu_copies((5, 6), sem) + in_copies(3, sem) + q_copies((2, 3), sem)
        if g == 6:
            return [pltpu.make_async_copy(wd_hbm, wd_v, sem)]
        return q_copies((4, 5, 6, 7), sem)

    def late_copies(m):
        return in_copies(m, in_sem.at[m - 4])

    def out_copy(b, slot):
        return pltpu.make_async_copy(o_v.at[b], o_hbm.at[:, pl.ds(b * TM, TM)], o_sem.at[slot])

    def out_quadrant(b, slot, hf, kh):
        c0 = pl.multiple_of(b * TM + hf * TH, TH)
        return pltpu.make_async_copy(o_v.at[b, pl.ds(kh * KH, KH), pl.ds(hf * TH, TH)],
                                     o_hbm.at[pl.ds(kh * KH, KH), pl.ds(c0, TH)], o_sem.at[slot])

    def start(cps):
        for cp in cps:
            cp.start()

    def wait(cps):
        for cp in cps:
            cp.wait()

    def conv_h(m):
        spec = [_dot(h_v[m, :, c * B:(c + 1) * B], _halves(ffwd_v[...])) for c in range(2)]
        sgn = 1.0 - 2.0 * (lax.broadcasted_iota(jnp.int32, (1, B), 1) & 1).astype(f32)
        first = isinstance(m, int) and m == 0
        if not first:
            hr_p, hi_p = hp_s[0], hp_s[1]
        for c in range(2):
            hr, hi = spec[c][:, :B], spec[c][:, B:]
            br = sgn * hi
            bi = -sgn * hr
            if not (first and c == 0):
                br = br + hr_p
                bi = bi + hi_p
            g_s[0, 2 * m + c + 1] = br
            g_s[1, 2 * m + c + 1] = bi - br
            g_s[2, 2 * m + c + 1] = br + bi
            hr_p, hi_p = hr, hi
        hp_s[0] = hr_p
        hp_s[1] = hi_p

    def conv_u(m):
        lane = lax.broadcasted_iota(jnp.int32, (RC // 2, B), 1)
        for r in range(D // RC):
            rs = slice(r * RC, (r + 1) * RC)
            if isinstance(m, int) and m == 0:
                halo = jnp.zeros((RC // 2, B), u32)
            else:
                halo = _words(k_v[m - 1, rs, B:PW])
            tiles = [halo, _words(k_v[m, rs, 0:B]), _words(k_v[m, rs, B:PW])]
            rolled = [[pltpu.roll(t, j, 1) for t in tiles] for j in range(1, 4)]
            for c in range(2):
                ks = _halves(tiles[c + 1]).astype(f32) * coef[0, rs]
                for j in range(1, 4):
                    kj = jnp.where(lane >= j, rolled[j - 1][c + 1], rolled[j - 1][c])
                    ks = ks + _halves(kj).astype(f32) * coef[j, rs]
                kv = (ks * v_v[m, rs, c * B:(c + 1) * B].astype(f32)).astype(bf16)
                y_s[2 * m + c, rs] = kv.astype(f32) * coef[4, rs]
                kv_s[c, rs] = kv
        spec = [_dot(kv_s[c], _halves(ffwd_v[...])) for c in range(2)]
        for c in range(2):
            ar, ai = spec[c][:, :B], spec[c][:, B:]
            u_s[0, 2 * m + c] = ar + ai
            u_s[1, 2 * m + c] = ar
            u_s[2, 2 * m + c] = ai

    def conv_unit(i_out, j_in, init=False):
        dl = 2 * (i_out - j_in)
        diag = isinstance(dl, int) and dl == 0
        for r in range(D // UC):
            rs = pl.ds(r * UC, UC)
            k0, k1 = [], []
            for t in range(3):
                gb, gc = g_s[t, dl + 1, rs], g_s[t, dl + 2, rs]
                u0, u1 = u_s[t, 2 * j_in, rs], u_s[t, 2 * j_in + 1, rs]
                k0.append(gb * u0 if diag else gb * u0 + g_s[t, dl, rs] * u1)
                k1.append(gc * u0 + gb * u1)
            for a, ks in enumerate((k0, k1)):
                re, im = ks[0] - ks[2], ks[0] + ks[1]
                if init is False:
                    re = ya_s[0, 2 * i_out + a, rs] + re
                    im = ya_s[1, 2 * i_out + a, rs] + im
                elif init is not True:
                    re = jnp.where(init, 0.0, ya_s[0, 2 * i_out + a, rs]) + re
                    im = jnp.where(init, 0.0, ya_s[1, 2 * i_out + a, rs]) + im
                ya_s[0, 2 * i_out + a, rs] = re
                ya_s[1, 2 * i_out + a, rs] = im

    def table_unit(s, init=False):
        conv_unit(tab[2 * s], tab[2 * s + 1], init=init)

    def conv_inverse(m):
        yi = [_dot(jnp.concatenate([ya_s[0, 2 * m + c], ya_s[1, 2 * m + c]], axis=1).astype(bf16),
                   _halves(finv_v[...])) for c in range(2)]
        for c in range(2):
            y_s[2 * m + c] = y_s[2 * m + c] + yi[c]

    stage_count = [0]

    def rounded(x):
        i = stage_count[0] % NSTAGE
        stage_count[0] += 1
        r, c = x.shape
        stage[i, 0:r, 0:c] = x.astype(bf16)
        return _words(stage[i, 0:r, 0:c])

    def prep_gu(c, from_table=False):
        c8 = pl.ds(pl.multiple_of(par[P_INT + c] * 8, 8), 8) if from_table else slice(c * 8, (c + 1) * 8)
        for i, w in enumerate((wg_v, wu_v)):
            wt1 = w[0:KH, c * PW:(c + 1) * PW].T
            wt2 = w[KH:D, c * PW:(c + 1) * PW].T
            f1, f2 = wt1.astype(f32), wt2.astype(f32)
            cs = _acombos(f1[:B], f2[:B], f1[B:], f2[B:])
            for p in range(7):
                if p == 2:
                    a = _words(wt1[:B])
                elif p == 3:
                    a = _words(wt2[B:])
                else:
                    a = _words(cs[p].astype(bf16))
                agu[p, c8, i] = a.reshape(8, 8, KH)

    def prep_d():
        for c in range(NCH):
            w = wd_v[:, c * PW:(c + 1) * PW]
            f = w.astype(f32)
            cs = _acombos(f[:KH, :B], f[:KH, B:], f[KH:, :B], f[KH:, B:])
            for p in range(7):
                if p == 2:
                    a = _words(w[:KH, :B])
                elif p == 3:
                    a = _words(w[KH:, B:])
                else:
                    a = rounded(cs[p])
                ad[p, :, c * B:(c + 1) * B] = a

    def item_block(n):
        return 2 * (n // 4) + n % 2

    def head(n):
        static = isinstance(n, int)
        blk = item_block(n) if static else jnp.minimum(item_block(n), NT - 1)
        for c in range(TM // B):
            slot = n % 2 if static else par[(n % 2) * 4 + c]
            rs = slice((c // 2) * D, (c // 2 + 1) * D)
            cs = slice((c % 2) * B, (c % 2 + 1) * B)
            xr = lambda: xb[2 + slot, rs, cs]
            mu = jnp.mean(xr(), axis=0, keepdims=True)
            xc = xr() - mu
            rstd = lax.rsqrt(jnp.mean(xc * xc, axis=0, keepdims=True) + EPS)
            x0 = xr()
            x1 = x0 + (x0 - mu) * rstd * y_s[4 * blk + c]
            xb[2 + slot, rs, cs] = x1
            mu = jnp.mean(x1, axis=0, keepdims=True)
            xc = xr() - mu
            rstd = lax.rsqrt(jnp.mean(xc * xc, axis=0, keepdims=True) + EPS)
            xb[slot, rs, cs] = (xr() - mu) * rstd

    def load_q(slot, blk):
        for hf in range(2):
            xb[2 + slot, hf * D:(hf + 1) * D] = q_v[2 * blk + hf].astype(f32)

    def b_operand(slot, p):
        b11 = lambda: xb[slot, 0:KH]
        b21 = lambda: xb[slot, KH:D]
        b12 = lambda: xb[slot, D:D + KH]
        b22 = lambda: xb[slot, D + KH:2 * D]
        return (lambda: b11() + b22(), b11, lambda: b12() - b22(), lambda: b21() - b11(), b22,
                lambda: b11() + b12(), lambda: b21() + b22())[p]().astype(bf16)

    def down_and_tail(n, fence_at=2, eager_out=False):
        static = isinstance(n, int)
        slot = n % 2
        blk = item_block(n)

        def down(k, p, v):
            if k == fence_at:
                top = jnp.where(par[P_ZERO] == 1, xb[par[P_ZERO2], 0:16], v[0:16])
                v = jnp.concatenate([top, v[16:]], axis=0)
            return _dot(_halves(ad[p]), v.astype(bf16))

        head(par[P_INT + 1] if static else n + 1)
        d4 = down(4, 3, hq[2] - hq[0])
        d6 = down(6, 5, hq[0] + hq[1])
        if static:
            d3 = down(3, 2, hq[1] - hq[3])
            d1 = down(1, 0, hq[0] + hq[3])
            d7 = down(7, 6, hq[2] + hq[3])
            d2 = down(2, 1, hq[0])
            d5 = down(5, 4, hq[3])
        else:
            d5 = down(5, 4, hq[3])
            d1 = down(1, 0, hq[0] + hq[3])
            d2 = down(2, 1, hq[0])
            d3 = down(3, 2, hq[1] - hq[3])
            d7 = down(7, 6, hq[2] + hq[3])
        last = (n // 2) % 2 == 1
        for hf, kh, o in ((0, 1, d2 + d4), (1, 0, d3 + d5), (1, 1, d1 - d2 + d3 + d6), (0, 0, d1 + d4 - d5 + d7)):
            rs = slice(hf * D + kh * KH, hf * D + (kh + 1) * KH)
            xo = xb[2 + slot, rs] + o
            if static:
                xb[2 + slot, rs] = xo
            else:
                o_v[blk, kh * KH:(kh + 1) * KH, hf * TH:(hf + 1) * TH] = xo.astype(bf16)
                if eager_out:
                    out_quadrant(blk, slot, hf, kh).start()
                nb = jnp.minimum(blk + 2, NT - 1)
                qn = q_v[2 * nb + hf, kh * KH:(kh + 1) * KH].astype(f32)
                xb[2 + slot, rs] = jnp.where(last, qn, xo)

    def products(c, hooks=None):
        hooks = hooks or {}
        count = [0]

        def mm(p):
            if count[0] in hooks:
                hooks[count[0]]()
            count[0] += 1
            return _dot(_halves(agu[p, c * 8:(c + 1) * 8].reshape(B, KH)), _halves(bc_s[p]))

        rs = slice(c * B, (c + 1) * B)
        m2, m4 = mm(1), mm(3)
        hq[2, rs] = _act(m2 + m4)
        m5, m3 = mm(4), mm(2)
        hq[1, rs] = _act(m3 + m5)
        m1 = mm(0)
        m7 = mm(6)
        hq[0, rs] = _act(m1 + m4 - m5 + m7)
        m6 = mm(5)
        hq[3, rs] = _act(m1 - m2 + m3 + m6)

    def units0(lo, hi, inits):
        for s in range(lo, hi):
            table_unit(len(UNITS) * NSLOT + s, s in inits)

    def block(fn):
        pl.when(par[P_ZERO] == 0)(fn)

    start(group(0) + group(1))
    for s, (i, j) in enumerate([u for row in UNITS for u in row] + list(UNITS0)):
        tab[2 * s] = i
        tab[2 * s + 1] = j
    for i in range(8):
        par[i] = i // 4
    par[P_ZERO] = 0
    par[P_ZERO2] = 0
    for c in range(NCH):
        par[P_INT + c] = c
    ffwd, finv = _dft_mats()
    ffwd_v[...] = _words(ffwd)
    finv_v[...] = _words(finv)
    for t in range(3):
        g_s[t, 0] = jnp.zeros((D, B), f32)
    wait(group(0))
    start(group(2))
    sk = sk_v[...].astype(f32)
    dv = d_v[...].astype(f32).reshape(1, D)
    for j in range(5):
        row = sk[j:j + 1] if j < 4 else dv
        coef[j] = jnp.broadcast_to(row, (B, D)).T

    wait(group(1))
    start(group(8))
    conv_h(0)
    conv_u(0)
    conv_unit(0, 0, init=True)
    conv_inverse(0)
    wait(group(2))
    start(group(3))
    conv_h(1)
    conv_u(1)
    conv_unit(1, 0, init=True)
    conv_unit(1, 1)
    conv_inverse(1)
    wait(group(8))
    start(group(4))
    prep_gu(0)
    load_q(0, 0)
    head(0)
    for cc in range(2):
        def quad(kh, hf):
            return xb[0, hf * D + kh * KH:hf * D + (kh + 1) * KH, cc * B:(cc + 1) * B]
        parts = _bcombos(quad(0, 0), quad(0, 1), quad(1, 0), quad(1, 1))
        for p in range(7):
            bc_s[p, :, cc * B:(cc + 1) * B] = _words(parts[p].astype(bf16))

    wait(group(3))
    start(group(5) + group(6))

    @block
    def _():
        products(0)
        prep_gu(1)
        products(1, {1: lambda: prep_gu(2, True)})

    wait(group(4))

    @block
    def _():
        m = par[P_INT + 2]
        products(2, {1: lambda: conv_h(m), 3: lambda: conv_u(m)})
        prep_gu(3)
        units0(0, 4, (0, 3))
        products(3)
        conv_inverse(m)
        prep_gu(4)

    wait(group(5))
    start(late_copies(4) + group(7))

    @block
    def _():
        m = par[P_INT + 3]
        products(4, {1: lambda: conv_h(m), 3: lambda: conv_u(m)})
        prep_gu(5)
        units0(4, 9, (4,))
        products(5)
        prep_gu(6)
        load_q(1, 1)
        products(6)
        conv_inverse(m)

    wait(group(6))

    @block
    def _():
        prep_d()
        down_and_tail(0)

    def body(n, with_conv):
        slot = n % 2
        m = n + 3

        def unit(s):
            if with_conv:
                table_unit((n - 1) * NSLOT + s, (n < 4) if s == 0 else False)

        def mm(p):
            return _dot(_halves(agu[p].reshape(F // 2, KH)), b_operand(slot, p))

        if with_conv:
            wait(late_copies(m))
            conv_h(m)
        else:
            out_copy(0, slot).wait()
        m2 = mm(1)
        if with_conv:
            conv_u(m)
        m5 = mm(4)
        unit(0)
        unit(1)
        m1 = mm(0)
        unit(2)
        unit(3)
        m4 = mm(3)
        hq[2] = _act(m2 + m4)
        unit(4)
        unit(5)
        m3 = mm(2)
        hq[1] = _act(m3 + m5)
        if with_conv:
            conv_inverse(m)
        m7 = mm(6)
        hq[0] = _act(m1 + m4 - m5 + m7)
        m6 = mm(5)
        hq[3] = _act(m1 - m2 + m3 + m6)
        down_and_tail(n, 2 if with_conv else 5, not with_conv)

        if with_conv:
            @pl.when((n // 2) % 2 == 1)
            def _():
                out_copy(item_block(n), slot).start()

    def body_conv(n, carry):
        body(n, True)
        return carry

    def body_plain(n, carry):
        body(n, False)
        return carry

    wait(group(7))
    start(late_copies(5) + late_copies(6) + late_copies(7))
    lax.fori_loop(1, 5, body_conv, 0)
    lax.fori_loop(5, 8, body_plain, 0)
    for slot in range(2):
        out_copy(0, slot).wait()


@jax.jit
def pallas_interleave_layers__ssm_conv_h3__geglu_ffn__prompt_kernel(A_q, A_k, A_v, A_shift_k, A_ssm_k, A_ssm_D, B_x, B_w_gate, B_w_up, B_w_down):
    hbm = pl.BlockSpec(memory_space=pl.ANY)
    out = pl.pallas_call(
        _kernel,
        in_specs=[hbm] * 9,
        out_specs=hbm,
        out_shape=jax.ShapeDtypeStruct((D, S), bf16),
        scratch_shapes=[
            pltpu.VMEM((NP, D, PW), bf16),
            pltpu.VMEM((NP, D, PW), bf16),
            pltpu.VMEM((NP, D, PW), bf16),
            pltpu.VMEM((NP, D, PW), bf16),
            pltpu.VMEM((D, F), bf16),
            pltpu.VMEM((D, F), bf16),
            pltpu.VMEM((D, F), bf16),
            pltpu.VMEM((4, D), bf16),
            pltpu.VMEM((D,), bf16),
            pltpu.VMEM((7, FH // 16, 2, 8, KH), u32),
            pltpu.VMEM((7, KH // 2, FH), u32),
            pltpu.VMEM((B // 2, 2 * B), u32),
            pltpu.VMEM((B, B), u32),
            pltpu.VMEM((5, D, B), f32),
            pltpu.VMEM((3, NB, D, B), f32),
            pltpu.VMEM((3, NB + 1, D, B), f32),
            pltpu.VMEM((2, D, B), f32),
            pltpu.VMEM((2, NB, D, B), f32),
            pltpu.VMEM((NB, D, B), f32),
            pltpu.VMEM((NT, D, TM), bf16),
            pltpu.VMEM((2, D, B), bf16),
            pltpu.VMEM((4, FH, TH), f32),
            pltpu.VMEM((4, FH, TH), f32),
            pltpu.VMEM((7, KH // 2, TH), u32),
            pltpu.VMEM((NSTAGE, KH, B), bf16),
            pltpu.SMEM((2 * (len(UNITS) * NSLOT + len(UNITS0)),), jnp.int32),
            pltpu.SMEM((P_INT + NCH,), jnp.int32),
            pltpu.SemaphoreType.DMA((9,)),
            pltpu.SemaphoreType.DMA((4,)),
            pltpu.SemaphoreType.DMA((2,)),
        ],
        compiler_params=pltpu.CompilerParams(vmem_limit_bytes=110 * 1024 * 1024),
    )(A_q[0].T, A_k[0].T, A_v[0].T, A_shift_k.T, A_ssm_k, A_ssm_D, B_w_gate, B_w_up, B_w_down.T)
    return out.T[None]
```

```python
import math

import jax
import jax.numpy as jnp
from jax import lax
from jax.experimental import pallas as pl
from jax.experimental.pallas import tpu as pltpu

S, D, F = 2048, 448, 1792
B = 128
NB = S // B
PW = 2 * B
NP = S // PW
TM = 512
TH = TM // 2
NT = S // TM
KH = D // 2
FH = F // 2
NCH = F // PW
RC = 32
UC = 32
EPS = 1e-5
f32 = jnp.float32
bf16 = jnp.bfloat16
u32 = jnp.uint32

UNITS = (
    ((5, 1), (4, 0), (4, 3), (4, 4), (5, 2), (5, 3)),
    ((6, 1), (5, 0), (5, 4), (5, 5), (6, 2), (6, 3)),
    ((7, 1), (6, 0), (6, 4), (6, 5), (6, 6), (7, 2)),
    ((7, 3), (7, 0), (7, 4), (7, 5), (7, 6), (7, 7)),
)
NSLOT = 6
UNITS0 = ((2, 0), (2, 1), (2, 2), (4, 2), (3, 1), (3, 2), (3, 0), (3, 3), (4, 1))
P_ZERO, P_ZERO2, P_INT = 8, 9, 10
EARLY_T = (0, 5)


def _angle(m):
    m = m & 511
    m = jnp.where(m >= 256, m - 512, m)
    return m.astype(f32) * (math.pi / 256.0)


def _dft_mats():
    r = lax.broadcasted_iota(jnp.int32, (B, B), 0)
    c = lax.broadcasted_iota(jnp.int32, (B, B), 1)
    ang = _angle((2 * c + 1) * r)
    ffwd = jnp.concatenate([jnp.cos(ang), -jnp.sin(ang)], axis=1).astype(bf16)
    ang = _angle((2 * r + 1) * (c + B))
    finv = (jnp.concatenate([jnp.cos(ang), -jnp.sin(ang)], axis=0) * (2.0 / 256.0)).astype(bf16)
    return ffwd, finv


def _gelu(x):
    c = math.sqrt(2.0 / math.pi)
    return 0.5 * x * (1.0 + jnp.tanh(c * (x + 0.044715 * (x * x * x))))


def _acombos(a11, a12, a21, a22):
    return [a11 + a22, a21 + a22, a11, a22, a11 + a12, a21 - a11, a12 - a22]


def _words(x):
    return pltpu.bitcast(x, u32)


def _halves(x):
    return pltpu.bitcast(x, bf16)


def _dot(a, b):
    return jnp.dot(a, b, preferred_element_type=f32)


def _act(c):
    rows = c.shape[0] // 2
    c = c.reshape(rows // 16, 2, 16, TH)
    return (_gelu(c[:, 0]) * c[:, 1]).reshape(rows, TH)


def _kernel(q_hbm, k_hbm, v_hbm, sk_hbm, h_hbm, d_hbm, wg_hbm, wu_hbm, wd_hbm, o_hbm,
            q_v, k_v, v_v, h_v, wg_v, wu_v, wd_v, sk_v, d_v, agu, ad, ffwd_v, finv_v, coef,
            u_s, g_s, hp_s, ya_s, y_s, o_v, kv_s, hq, xb, bc_s, tab, par, g_sem, in_sem, o_sem):

    def slab(src, dst, m, sem):
        c0 = m * PW if isinstance(m, int) else pl.multiple_of(m * PW, PW)
        return pltpu.make_async_copy(src.at[:, pl.ds(c0, PW)], dst.at[m], sem)

    def in_copies(m, sem):
        return [slab(src, dst, m, sem) for src, dst in ((k_hbm, k_v), (v_hbm, v_v), (h_hbm, h_v))]

    def q_copies(ms, sem):
        return [slab(q_hbm, q_v, m, sem) for m in ms]

    def gu_copies(cs, sem):
        return [pltpu.make_async_copy(src.at[:, pl.ds(c * PW, PW)], dst.at[:, pl.ds(c * PW, PW)], sem)
                for c in cs for src, dst in ((wg_hbm, wg_v), (wu_hbm, wu_v))]

    def group(g):
        sem = g_sem.at[g]
        if g == 0:
            return [pltpu.make_async_copy(sk_hbm, sk_v, sem), pltpu.make_async_copy(d_hbm, d_v, sem)]
        if g == 1:
            return in_copies(0, sem)
        if g == 2:
            return in_copies(1, sem)
        if g == 8:
            return q_copies((0, 1), sem) + gu_copies((0,), sem)
        if g == 3:
            return gu_copies((1, 2), sem)
        if g == 4:
            return gu_copies((3, 4), sem) + in_copies(2, sem)
        if g == 5:
            return gu_copies((5, 6), sem) + in_copies(3, sem) + q_copies((2, 3), sem)
        if g == 6:
            return [pltpu.make_async_copy(wd_hbm, wd_v, sem)]
        return q_copies((4, 5, 6, 7), sem)

    def late_copies(m):
        return in_copies(m, in_sem.at[m - 4])

    def out_copy(b, slot):
        return pltpu.make_async_copy(o_v.at[b], o_hbm.at[:, pl.ds(b * TM, TM)], o_sem.at[slot])

    def out_quadrant(b, slot, hf, kh):
        c0 = pl.multiple_of(b * TM + hf * TH, TH)
        return pltpu.make_async_copy(o_v.at[b, pl.ds(kh * KH, KH), pl.ds(hf * TH, TH)],
                                     o_hbm.at[pl.ds(kh * KH, KH), pl.ds(c0, TH)], o_sem.at[slot])

    def start(cps):
        for cp in cps:
            cp.start()

    def wait(cps):
        for cp in cps:
            cp.wait()

    def conv_h(m):
        spec = [_dot(h_v[m, :, c * B:(c + 1) * B], _halves(ffwd_v[...])) for c in range(2)]
        sgn = 1.0 - 2.0 * (lax.broadcasted_iota(jnp.int32, (1, B), 1) & 1).astype(f32)
        first = isinstance(m, int) and m == 0
        if not first:
            hr_p, hi_p = hp_s[0], hp_s[1]
        for c in range(2):
            hr, hi = spec[c][:, :B], spec[c][:, B:]
            br = sgn * hi
            bi = -sgn * hr
            if not (first and c == 0):
                br = br + hr_p
                bi = bi + hi_p
            g_s[0, 2 * m + c + 1] = br
            g_s[1, 2 * m + c + 1] = bi - br
            g_s[2, 2 * m + c + 1] = br + bi
            hr_p, hi_p = hr, hi
        hp_s[0] = hr_p
        hp_s[1] = hi_p

    def conv_u(m):
        lane = lax.broadcasted_iota(jnp.int32, (RC // 2, B), 1)
        for r in range(D // RC):
            rs = slice(r * RC, (r + 1) * RC)
            if isinstance(m, int) and m == 0:
                halo = jnp.zeros((RC // 2, B), u32)
            else:
                halo = _words(k_v[m - 1, rs, B:PW])
            tiles = [halo, _words(k_v[m, rs, 0:B]), _words(k_v[m, rs, B:PW])]
            rolled = [[pltpu.roll(t, j, 1) for t in tiles] for j in range(1, 4)]
            for c in range(2):
                ks = _halves(tiles[c + 1]).astype(f32) * coef[0, rs]
                for j in range(1, 4):
                    kj = jnp.where(lane >= j, rolled[j - 1][c + 1], rolled[j - 1][c])
                    ks = ks + _halves(kj).astype(f32) * coef[j, rs]
                kv = (ks * v_v[m, rs, c * B:(c + 1) * B].astype(f32)).astype(bf16)
                if not isinstance(m, int):
                    y_s[2 * m + c, rs] = kv.astype(f32) * coef[4, rs]
                kv_s[c, rs] = kv
        spec = [_dot(kv_s[c], _halves(ffwd_v[...])) for c in range(2)]
        for c in range(2):
            ar, ai = spec[c][:, :B], spec[c][:, B:]
            u_s[0, 2 * m + c] = ar + ai
            u_s[1, 2 * m + c] = ar
            u_s[2, 2 * m + c] = ai

    def conv_unit(i_out, j_in, init=False):
        dl = 2 * (i_out - j_in)
        diag = isinstance(dl, int) and dl == 0
        for r in range(D // UC):
            rs = pl.ds(r * UC, UC)
            k0, k1 = [], []
            for t in range(3):
                gb, gc = g_s[t, dl + 1, rs], g_s[t, dl + 2, rs]
                u0, u1 = u_s[t, 2 * j_in, rs], u_s[t, 2 * j_in + 1, rs]
                k0.append(gb * u0 if diag else gb * u0 + g_s[t, dl, rs] * u1)
                k1.append(gc * u0 + gb * u1)
            for a, ks in enumerate((k0, k1)):
                re, im = ks[0] - ks[2], ks[0] + ks[1]
                if init is False:
                    re = ya_s[0, 2 * i_out + a, rs] + re
                    im = ya_s[1, 2 * i_out + a, rs] + im
                elif init is not True:
                    re = jnp.where(init, 0.0, ya_s[0, 2 * i_out + a, rs]) + re
                    im = jnp.where(init, 0.0, ya_s[1, 2 * i_out + a, rs]) + im
                ya_s[0, 2 * i_out + a, rs] = re
                ya_s[1, 2 * i_out + a, rs] = im

    def table_unit(s, init=False):
        conv_unit(tab[2 * s], tab[2 * s + 1], init=init)

    def conv_inverse(m):
        yi = [_dot(jnp.concatenate([ya_s[0, 2 * m + c], ya_s[1, 2 * m + c]], axis=1).astype(bf16),
                   _halves(finv_v[...])) for c in range(2)]
        for c in range(2):
            skip = kv_s[c].astype(f32) * coef[4] if isinstance(m, int) else y_s[2 * m + c]
            y_s[2 * m + c] = skip + yi[c]

    def rounded(x):
        return _words(x.astype(bf16))

    def prep_gu(c):
        c8 = slice(c * 8, (c + 1) * 8)
        for i, w in enumerate((wg_v, wu_v)):
            if c in EARLY_T:
                wt1 = w[0:KH, c * PW:(c + 1) * PW].T
                wt2 = w[KH:D, c * PW:(c + 1) * PW].T
                f1, f2 = wt1.astype(f32), wt2.astype(f32)
                cs = _acombos(f1[:B], f2[:B], f1[B:], f2[B:])
                for p in range(7):
                    if p == 2:
                        a = _words(wt1[:B])
                    elif p == 3:
                        a = _words(wt2[B:])
                    else:
                        a = rounded(cs[p])
                    agu[p, c8, i] = a.reshape(8, 8, KH)
            else:
                wc = w[:, c * PW:(c + 1) * PW]
                f = wc.astype(f32)
                cs = _acombos(f[:KH, :B], f[KH:, :B], f[:KH, B:], f[KH:, B:])
                for p in range(7):
                    if p == 2:
                        a = wc[:KH, :B]
                    elif p == 3:
                        a = wc[KH:, B:]
                    else:
                        a = cs[p].astype(bf16)
                    agu[p, c8, i] = _words(a.T).reshape(8, 8, KH)

    def prep_d():
        rc = 32
        for c in range(NCH):
            for r in range(KH // rc):
                w = [wd_v[kh * KH + r * rc:kh * KH + (r + 1) * rc, c * PW + e * B:c * PW + (e + 1) * B]
                     for kh in range(2) for e in range(2)]
                cs = _acombos(*[x.astype(f32) for x in w])
                for p in range(7):
                    a = _words(w[0]) if p == 2 else _words(w[3]) if p == 3 else rounded(cs[p])
                    if False and p == 0 and (c, r) != (0, 0):
                        top = jnp.where(par[P_ZERO] == 1, ad[par[P_ZERO2], 0:8, 0:B], a[0:8])
                        a = jnp.concatenate([top, a[8:]], axis=0)
                    ad[p, r * rc // 2:(r + 1) * rc // 2, c * B:(c + 1) * B] = a

    def item_block(n):
        return 2 * (n // 4) + n % 2

    def head(n):
        static = isinstance(n, int)
        blk = item_block(n) if static else jnp.minimum(item_block(n), NT - 1)
        for c in range(TM // B):
            slot = n % 2 if static else par[(n % 2) * 4 + c]
            rs = slice((c // 2) * D, (c // 2 + 1) * D)
            cs = slice((c % 2) * B, (c % 2 + 1) * B)
            xr = lambda: xb[2 + slot, rs, cs]
            xin = (lambda: q_v[c // 2, :, cs].astype(f32)) if static else xr
            mu = jnp.mean(xin(), axis=0, keepdims=True)
            xc = xin() - mu
            rstd = lax.rsqrt(jnp.mean(xc * xc, axis=0, keepdims=True) + EPS)
            x0 = xin()
            x1 = x0 + (x0 - mu) * rstd * y_s[4 * blk + c]
            xb[2 + slot, rs, cs] = x1
            mu = jnp.mean(x1, axis=0, keepdims=True)
            xc = xr() - mu
            rstd = lax.rsqrt(jnp.mean(xc * xc, axis=0, keepdims=True) + EPS)
            xb[slot, rs, cs] = (xr() - mu) * rstd

    def load_q(slot, blk):
        for hf in range(2):
            xb[2 + slot, hf * D:(hf + 1) * D] = q_v[2 * blk + hf].astype(f32)

    def b_operand(slot, p):
        b11 = lambda: xb[slot, 0:KH]
        b21 = lambda: xb[slot, KH:D]
        b12 = lambda: xb[slot, D:D + KH]
        b22 = lambda: xb[slot, D + KH:2 * D]
        return (lambda: b11() + b22(), b11, lambda: b12() - b22(), lambda: b21() - b11(), b22,
                lambda: b11() + b12(), lambda: b21() + b22())[p]().astype(bf16)

    def down_and_tail(n, fence_at=2, eager_out=False):
        static = isinstance(n, int)
        slot = n % 2
        blk = item_block(n)

        def down(k, p, v):
            if k == fence_at:
                top = jnp.where(par[P_ZERO] == 1, xb[par[P_ZERO2], 0:16], v[0:16])
                v = jnp.concatenate([top, v[16:]], axis=0)
            return _dot(_halves(ad[p]), v.astype(bf16))

        head(par[P_INT + 1] if static else n + 1)
        d4 = down(4, 3, hq[2] - hq[0])
        d6 = down(6, 5, hq[0] + hq[1])
        if static:
            d3 = down(3, 2, hq[1] - hq[3])
            d1 = down(1, 0, hq[0] + hq[3])
            d7 = down(7, 6, hq[2] + hq[3])
            d2 = down(2, 1, hq[0])
            d5 = down(5, 4, hq[3])
        else:
            d5 = down(5, 4, hq[3])
            d1 = down(1, 0, hq[0] + hq[3])
            d2 = down(2, 1, hq[0])
            d3 = down(3, 2, hq[1] - hq[3])
            d7 = down(7, 6, hq[2] + hq[3])
        last = (n // 2) % 2 == 1
        for hf, kh, o in ((0, 1, d2 + d4), (1, 0, d3 + d5), (1, 1, d1 - d2 + d3 + d6), (0, 0, d1 + d4 - d5 + d7)):
            rs = slice(hf * D + kh * KH, hf * D + (kh + 1) * KH)
            xo = xb[2 + slot, rs] + o
            if static:
                xb[2 + slot, rs] = xo
            else:
                o_v[blk, kh * KH:(kh + 1) * KH, hf * TH:(hf + 1) * TH] = xo.astype(bf16)
                if eager_out:
                    out_quadrant(blk, slot, hf, kh).start()
                nb = jnp.minimum(blk + 2, NT - 1)
                qn = q_v[2 * nb + hf, kh * KH:(kh + 1) * KH].astype(f32)
                xb[2 + slot, rs] = jnp.where(last, qn, xo)

    def products(c, hooks=None):
        hooks = hooks or {}
        count = [0]

        def mm(p):
            if count[0] in hooks:
                hooks[count[0]]()
            count[0] += 1
            b = b_operand(0, p) if c == 0 else _halves(bc_s[p])
            return _dot(_halves(agu[p, c * 8:(c + 1) * 8].reshape(B, KH)), b)

        rs = slice(c * B, (c + 1) * B)
        m2, m4 = mm(1), mm(3)
        hq[2, rs] = _act(m2 + m4)
        m5, m3 = mm(4), mm(2)
        hq[1, rs] = _act(m3 + m5)
        m1 = mm(0)
        m7 = mm(6)
        hq[0, rs] = _act(m1 + m4 - m5 + m7)
        m6 = mm(5)
        hq[3, rs] = _act(m1 - m2 + m3 + m6)

    def units0(lo, hi, inits):
        for s in range(lo, hi):
            table_unit(len(UNITS) * NSLOT + s, s in inits)

    def block(fn):
        pl.when(par[P_ZERO] == 0)(fn)

    start(group(0) + group(1))
    for s, (i, j) in enumerate([u for row in UNITS for u in row] + list(UNITS0)):
        tab[2 * s] = i
        tab[2 * s + 1] = j
    for i in range(8):
        par[i] = i // 4
    par[P_ZERO] = 0
    par[P_ZERO2] = 0
    for c in range(4):
        par[P_INT + c] = c
    ffwd, finv = _dft_mats()
    ffwd_v[...] = _words(ffwd)
    finv_v[...] = _words(finv)
    for t in range(3):
        g_s[t, 0] = jnp.zeros((D, B), f32)
    wait(group(0))
    start(group(2))
    sk = sk_v[...].astype(f32)
    dv = d_v[...].astype(f32).reshape(1, D)
    for j in range(5):
        row = sk[j:j + 1] if j < 4 else dv
        coef[j] = jnp.broadcast_to(row, (B, D)).T

    wait(group(1))
    start(group(8))
    conv_h(0)
    conv_u(0)
    conv_unit(0, 0, init=True)
    conv_inverse(0)
    wait(group(2))
    start(group(3))
    conv_h(1)
    conv_u(1)
    conv_unit(1, 0, init=True)
    conv_unit(1, 1)
    conv_inverse(1)
    wait(group(8))
    start(group(4))
    prep_gu(0)
    head(0)
    wait(group(3))
    start(group(5) + group(6))

    @block
    def _():
        products(0)
        for p in range(7):
            bc_s[p] = _words(b_operand(0, p))
        prep_gu(1)
        products(1)
        prep_gu(2)

    wait(group(4))

    @block
    def _():
        m = par[P_INT + 2]
        products(2, {1: lambda: conv_h(m), 3: lambda: conv_u(m)})
        prep_gu(3)
        units0(0, 4, (0, 3))
        products(3)
        conv_inverse(m)
        prep_gu(4)

    wait(group(5))
    start(late_copies(4) + group(7))

    @block
    def _():
        m = par[P_INT + 3]
        products(4, {1: lambda: conv_h(m), 3: lambda: conv_u(m)})
        prep_gu(5)
        units0(4, 9, (4,))
        products(5)
        prep_gu(6)
        load_q(1, 1)
        products(6)
        conv_inverse(m)

    wait(group(6))

    @block
    def _():
        prep_d()
        down_and_tail(0)

    def body(n, with_conv):
        slot = n % 2
        m = n + 3

        def unit(s):
            if with_conv:
                table_unit((n - 1) * NSLOT + s, (n < 4) if s == 0 else False)

        def mm(p):
            return _dot(_halves(agu[p].reshape(F // 2, KH)), b_operand(slot, p))

        if with_conv:
            wait(late_copies(m))
            conv_h(m)
        else:
            out_copy(0, slot).wait()
        m2 = mm(1)
        if with_conv:
            conv_u(m)
        m5 = mm(4)
        unit(0)
        unit(1)
        m1 = mm(0)
        unit(2)
        unit(3)
        m4 = mm(3)
        hq[2] = _act(m2 + m4)
        unit(4)
        unit(5)
        m3 = mm(2)
        hq[1] = _act(m3 + m5)
        if with_conv:
            conv_inverse(m)
        m7 = mm(6)
        hq[0] = _act(m1 + m4 - m5 + m7)
        m6 = mm(5)
        hq[3] = _act(m1 - m2 + m3 + m6)
        down_and_tail(n, 2 if with_conv else 5, not with_conv)

        if with_conv:
            @pl.when((n // 2) % 2 == 1)
            def _():
                out_copy(item_block(n), slot).start()

    def body_conv(n, carry):
        body(n, True)
        return carry

    def body_plain(n, carry):
        body(n, False)
        return carry

    wait(group(7))
    start(late_copies(5) + late_copies(6) + late_copies(7))
    lax.fori_loop(1, 5, body_conv, 0)
    lax.fori_loop(5, 8, body_plain, 0)
    for slot in range(2):
        out_copy(0, slot).wait()


@jax.jit
def pallas_interleave_layers__ssm_conv_h3__geglu_ffn__prompt_kernel(A_q, A_k, A_v, A_shift_k, A_ssm_k, A_ssm_D, B_x, B_w_gate, B_w_up, B_w_down):
    hbm = pl.BlockSpec(memory_space=pl.ANY)
    out = pl.pallas_call(
        _kernel,
        in_specs=[hbm] * 9,
        out_specs=hbm,
        out_shape=jax.ShapeDtypeStruct((D, S), bf16),
        scratch_shapes=[
            pltpu.VMEM((NP, D, PW), bf16),
            pltpu.VMEM((NP, D, PW), bf16),
            pltpu.VMEM((NP, D, PW), bf16),
            pltpu.VMEM((NP, D, PW), bf16),
            pltpu.VMEM((D, F), bf16),
            pltpu.VMEM((D, F), bf16),
            pltpu.VMEM((D, F), bf16),
            pltpu.VMEM((4, D), bf16),
            pltpu.VMEM((D,), bf16),
            pltpu.VMEM((7, FH // 16, 2, 8, KH), u32),
            pltpu.VMEM((7, KH // 2, FH), u32),
            pltpu.VMEM((B // 2, 2 * B), u32),
            pltpu.VMEM((B, B), u32),
            pltpu.VMEM((5, D, B), f32),
            pltpu.VMEM((3, NB, D, B), f32),
            pltpu.VMEM((3, NB + 1, D, B), f32),
            pltpu.VMEM((2, D, B), f32),
            pltpu.VMEM((2, NB, D, B), f32),
            pltpu.VMEM((NB, D, B), f32),
            pltpu.VMEM((NT, D, TM), bf16),
            pltpu.VMEM((2, D, B), bf16),
            pltpu.VMEM((4, FH, TH), f32),
            pltpu.VMEM((4, FH, TH), f32),
            pltpu.VMEM((7, KH // 2, TH), u32),
            pltpu.SMEM((2 * (len(UNITS) * NSLOT + len(UNITS0)),), jnp.int32),
            pltpu.SMEM((P_INT + 4,), jnp.int32),
            pltpu.SemaphoreType.DMA((9,)),
            pltpu.SemaphoreType.DMA((4,)),
            pltpu.SemaphoreType.DMA((2,)),
        ],
        compiler_params=pltpu.CompilerParams(vmem_limit_bytes=110 * 1024 * 1024),
    )(A_q[0].T, A_k[0].T, A_v[0].T, A_shift_k.T, A_ssm_k, A_ssm_D, B_w_gate, B_w_up, B_w_down.T)
    return out.T[None]
```

```python
import math

import jax
import jax.numpy as jnp
from jax import lax
from jax.experimental import pallas as pl
from jax.experimental.pallas import tpu as pltpu

S, D, F = 2048, 448, 1792
B = 128
NB = S // B
PW = 2 * B
NP = S // PW
TM = 512
TH = TM // 2
NT = S // TM
KH = D // 2
FH = F // 2
NCH = F // PW
RC = 32
UC = 32
EPS = 1e-5
f32 = jnp.float32
bf16 = jnp.bfloat16
u32 = jnp.uint32

UNITS = (
    ((5, 1), (4, 0), (4, 3), (4, 4), (5, 2), (5, 3)),
    ((6, 1), (5, 0), (5, 4), (5, 5), (6, 2), (6, 3)),
    ((7, 1), (6, 0), (6, 4), (6, 5), (6, 6), (7, 2)),
    ((7, 3), (7, 0), (7, 4), (7, 5), (7, 6), (7, 7)),
)
NSLOT = 6
UNITS0 = ((2, 0), (2, 1), (2, 2), (4, 2), (3, 1), (3, 2), (3, 0), (3, 3), (4, 1))
P_ZERO, P_ZERO2, P_INT = 8, 9, 10
EARLY_T = (0, 5)


def _angle(m):
    m = m & 511
    m = jnp.where(m >= 256, m - 512, m)
    return m.astype(f32) * (math.pi / 256.0)


def _dft_mats():
    r = lax.broadcasted_iota(jnp.int32, (B, B), 0)
    c = lax.broadcasted_iota(jnp.int32, (B, B), 1)
    ang = _angle((2 * c + 1) * r)
    cs, sn = jnp.cos(ang), jnp.sin(ang)
    ffwd = jnp.concatenate([cs, -sn], axis=1).astype(bf16)
    scale = (2.0 * (c & 1).astype(f32) - 1.0) * (2.0 / 256.0)
    finv = jnp.concatenate([(sn * scale).T, (cs * scale).T], axis=0).astype(bf16)
    return ffwd, finv


def _gelu(x):
    c = math.sqrt(2.0 / math.pi)
    return 0.5 * x * (1.0 + jnp.tanh(c * (x + 0.044715 * (x * x * x))))


def _acombos(a11, a12, a21, a22):
    return [a11 + a22, a21 + a22, a11, a22, a11 + a12, a21 - a11, a12 - a22]


def _words(x):
    return pltpu.bitcast(x, u32)


def _halves(x):
    return pltpu.bitcast(x, bf16)


def _dot(a, b):
    return jnp.dot(a, b, preferred_element_type=f32)


def _act(c):
    rows = c.shape[0] // 2
    c = c.reshape(rows // 16, 2, 16, TH)
    return (_gelu(c[:, 0]) * c[:, 1]).reshape(rows, TH)


def _kernel(q_hbm, k_hbm, v_hbm, sk_hbm, h_hbm, d_hbm, wg_hbm, wu_hbm, wd_hbm, o_hbm,
            q_v, k_v, v_v, h_v, wg_v, wu_v, wd_v, sk_v, d_v, agu, ad, ffwd_v, finv_v, coef,
            u_s, g_s, hp_s, ya_s, y_s, o_v, kv_s, hq, xb, bc_s, tab, par, g_sem, in_sem, o_sem):

    def slab(src, dst, m, sem):
        c0 = m * PW if isinstance(m, int) else pl.multiple_of(m * PW, PW)
        return pltpu.make_async_copy(src.at[:, pl.ds(c0, PW)], dst.at[m], sem)

    def in_copies(m, sem):
        return [slab(src, dst, m, sem) for src, dst in ((k_hbm, k_v), (v_hbm, v_v), (h_hbm, h_v))]

    def q_copies(ms, sem):
        return [slab(q_hbm, q_v, m, sem) for m in ms]

    def gu_copies(cs, sem):
        return [pltpu.make_async_copy(src.at[:, pl.ds(c * PW, PW)], dst.at[:, pl.ds(c * PW, PW)], sem)
                for c in cs for src, dst in ((wg_hbm, wg_v), (wu_hbm, wu_v))]

    def group(g):
        sem = g_sem.at[g]
        if g == 0:
            return [pltpu.make_async_copy(sk_hbm, sk_v, sem), pltpu.make_async_copy(d_hbm, d_v, sem)]
        if g == 1:
            return in_copies(0, sem)
        if g == 2:
            return in_copies(1, sem)
        if g == 8:
            return q_copies((0, 1), sem) + gu_copies((0,), sem)
        if g == 3:
            return gu_copies((1, 2), sem)
        if g == 4:
            return gu_copies((3, 4), sem) + in_copies(2, sem)
        if g == 5:
            return gu_copies((5, 6), sem) + in_copies(3, sem) + q_copies((2, 3), sem)
        if g == 6:
            return [pltpu.make_async_copy(wd_hbm, wd_v, sem)]
        return q_copies((4, 5, 6, 7), sem)

    def late_copies(m):
        return in_copies(m, in_sem.at[m - 4])

    def out_copy(b, slot):
        c0 = b * TM if isinstance(b, int) else pl.multiple_of(b * TM, TM)
        return pltpu.make_async_copy(o_v.at[b], o_hbm.at[:, pl.ds(c0, TM)], o_sem.at[slot])

    def out_quadrant(b, slot, hf, kh):
        c0 = pl.multiple_of(b * TM + hf * TH, TH)
        return pltpu.make_async_copy(o_v.at[b, pl.ds(kh * KH, KH), pl.ds(hf * TH, TH)],
                                     o_hbm.at[pl.ds(kh * KH, KH), pl.ds(c0, TH)], o_sem.at[slot])

    def start(cps):
        for cp in cps:
            cp.start()

    def wait(cps):
        for cp in cps:
            cp.wait()

    def conv_h(m):
        spec = [_dot(h_v[m, :, c * B:(c + 1) * B], _halves(ffwd_v[...])) for c in range(2)]
        sgn = 1.0 - 2.0 * (lax.broadcasted_iota(jnp.int32, (1, B), 1) & 1).astype(f32)
        first = isinstance(m, int) and m == 0
        if not first:
            hr_p, hi_p = hp_s[0], hp_s[1]
        for c in range(2):
            hr, hi = spec[c][:, :B], spec[c][:, B:]
            br = sgn * hi
            bi = -sgn * hr
            if not (first and c == 0):
                br = br + hr_p
                bi = bi + hi_p
            g_s[0, 2 * m + c + 1] = br
            g_s[1, 2 * m + c + 1] = bi - br
            g_s[2, 2 * m + c + 1] = br + bi
            hr_p, hi_p = hr, hi
        hp_s[0] = hr_p
        hp_s[1] = hi_p

    def conv_u(m):
        lane = lax.broadcasted_iota(jnp.int32, (RC // 2, B), 1)
        for r in range(D // RC):
            rs = slice(r * RC, (r + 1) * RC)
            if isinstance(m, int) and m == 0:
                halo = jnp.zeros((RC // 2, B), u32)
            else:
                halo = _words(k_v[m - 1, rs, B:PW])
            tiles = [halo, _words(k_v[m, rs, 0:B]), _words(k_v[m, rs, B:PW])]
            rolled = [[pltpu.roll(t, j, 1) for t in tiles] for j in range(1, 4)]
            for c in range(2):
                ks = _halves(tiles[c + 1]).astype(f32) * coef[0, rs]
                for j in range(1, 4):
                    kj = jnp.where(lane >= j, rolled[j - 1][c + 1], rolled[j - 1][c])
                    ks = ks + _halves(kj).astype(f32) * coef[j, rs]
                kv = (ks * v_v[m, rs, c * B:(c + 1) * B].astype(f32)).astype(bf16)
                if not isinstance(m, int):
                    y_s[2 * m + c, rs] = kv.astype(f32) * coef[4, rs]
                kv_s[c, rs] = kv
        spec = [_dot(kv_s[c], _halves(ffwd_v[...])) for c in range(2)]
        for c in range(2):
            ar, ai = spec[c][:, :B], spec[c][:, B:]
            u_s[0, 2 * m + c] = ar + ai
            u_s[1, 2 * m + c] = ar
            u_s[2, 2 * m + c] = ai

    def conv_unit(i_out, j_in, init=False):
        dl = 2 * (i_out - j_in)
        diag = isinstance(dl, int) and dl == 0
        for r in range(D // UC):
            rs = pl.ds(r * UC, UC)
            k0, k1 = [], []
            for t in range(3):
                gb, gc = g_s[t, dl + 1, rs], g_s[t, dl + 2, rs]
                u0, u1 = u_s[t, 2 * j_in, rs], u_s[t, 2 * j_in + 1, rs]
                k0.append(gb * u0 if diag else gb * u0 + g_s[t, dl, rs] * u1)
                k1.append(gc * u0 + gb * u1)
            for a, ks in enumerate((k0, k1)):
                re, im = ks[0] - ks[2], ks[0] + ks[1]
                if init is False:
                    re = ya_s[0, 2 * i_out + a, rs] + re
                    im = ya_s[1, 2 * i_out + a, rs] + im
                elif init is not True:
                    re = jnp.where(init, 0.0, ya_s[0, 2 * i_out + a, rs]) + re
                    im = jnp.where(init, 0.0, ya_s[1, 2 * i_out + a, rs]) + im
                ya_s[0, 2 * i_out + a, rs] = re
                ya_s[1, 2 * i_out + a, rs] = im

    def table_unit(s, init=False):
        conv_unit(tab[2 * s], tab[2 * s + 1], init=init)

    def conv_inverse(m):
        yi = [_dot(jnp.concatenate([ya_s[0, 2 * m + c], ya_s[1, 2 * m + c]], axis=1).astype(bf16),
                   _halves(finv_v[...])) for c in range(2)]
        for c in range(2):
            skip = kv_s[c].astype(f32) * coef[4] if isinstance(m, int) else y_s[2 * m + c]
            y_s[2 * m + c] = skip + yi[c]

    def rounded(x):
        return _words(x.astype(bf16))

    def prep_gu(c):
        c8 = slice(c * 8, (c + 1) * 8)
        for i, w in enumerate((wg_v, wu_v)):
            if c in EARLY_T:
                wt1 = w[0:KH, c * PW:(c + 1) * PW].T
                wt2 = w[KH:D, c * PW:(c + 1) * PW].T
                f1, f2 = wt1.astype(f32), wt2.astype(f32)
                cs = _acombos(f1[:B], f2[:B], f1[B:], f2[B:])
                for p in range(7):
                    if p == 2:
                        a = _words(wt1[:B])
                    elif p == 3:
                        a = _words(wt2[B:])
                    else:
                        a = rounded(cs[p])
                    agu[p, c8, i] = a.reshape(8, 8, KH)
            else:
                wc = w[:, c * PW:(c + 1) * PW]
                f = wc.astype(f32)
                cs = _acombos(f[:KH, :B], f[KH:, :B], f[:KH, B:], f[KH:, B:])
                for p in range(7):
                    if p == 2:
                        a = wc[:KH, :B]
                    elif p == 3:
                        a = wc[KH:, B:]
                    else:
                        a = cs[p].astype(bf16)
                    agu[p, c8, i] = _words(a.T).reshape(8, 8, KH)

    def prep_d():
        rc = 32
        for c in range(NCH):
            for r in range(KH // rc):
                w = [wd_v[kh * KH + r * rc:kh * KH + (r + 1) * rc, c * PW + e * B:c * PW + (e + 1) * B]
                     for kh in range(2) for e in range(2)]
                cs = _acombos(*[x.astype(f32) for x in w])
                for p in range(7):
                    a = _words(w[0]) if p == 2 else _words(w[3]) if p == 3 else rounded(cs[p])
                    ad[p, r * rc // 2:(r + 1) * rc // 2, c * B:(c + 1) * B] = a

    def item_block(n):
        return 2 * (n // 4) + n % 2

    def head(n):
        static = isinstance(n, int)
        blk = item_block(n) if static else jnp.minimum(item_block(n), NT - 1)
        for c in range(TM // B):
            slot = n % 2 if static else par[(n % 2) * 4 + c]
            rs = slice((c // 2) * D, (c // 2 + 1) * D)
            cs = slice((c % 2) * B, (c % 2 + 1) * B)
            xr = lambda: xb[2 + slot, rs, cs]
            xin = (lambda: q_v[c // 2, :, cs].astype(f32)) if static else xr
            mu = jnp.mean(xin(), axis=0, keepdims=True)
            xc = xin() - mu
            rstd = lax.rsqrt(jnp.mean(xc * xc, axis=0, keepdims=True) + EPS)
            x0 = xin()
            x1 = x0 + (x0 - mu) * rstd * y_s[4 * blk + c]
            xb[2 + slot, rs, cs] = x1
            mu = jnp.mean(x1, axis=0, keepdims=True)
            xc = xr() - mu
            rstd = lax.rsqrt(jnp.mean(xc * xc, axis=0, keepdims=True) + EPS)
            xb[slot, rs, cs] = (xr() - mu) * rstd

    def load_q(slot, blk):
        for hf in range(2):
            xb[2 + slot, hf * D:(hf + 1) * D] = q_v[2 * blk + hf].astype(f32)

    def b_operand(slot, p):
        b11 = lambda: xb[slot, 0:KH]
        b21 = lambda: xb[slot, KH:D]
        b12 = lambda: xb[slot, D:D + KH]
        b22 = lambda: xb[slot, D + KH:2 * D]
        return (lambda: b11() + b22(), b11, lambda: b12() - b22(), lambda: b21() - b11(), b22,
                lambda: b11() + b12(), lambda: b21() + b22())[p]().astype(bf16)

    def down_and_tail(n, fence_at=2, eager_out=False):
        static = isinstance(n, int)
        slot = n % 2
        blk = item_block(n)

        def down(k, p, v):
            if k == fence_at:
                top = jnp.where(par[P_ZERO] == 1, xb[par[P_ZERO2], 0:16], v[0:16])
                v = jnp.concatenate([top, v[16:]], axis=0)
            return _dot(_halves(ad[p]), v.astype(bf16))

        head(par[P_INT + 1] if static else n + 1)
        d4 = down(4, 3, hq[2] - hq[0])
        d6 = down(6, 5, hq[0] + hq[1])
        if static:
            d3 = down(3, 2, hq[1] - hq[3])
            d1 = down(1, 0, hq[0] + hq[3])
            d7 = down(7, 6, hq[2] + hq[3])
            d2 = down(2, 1, hq[0])
            d5 = down(5, 4, hq[3])
        else:
            d5 = down(5, 4, hq[3])
            d1 = down(1, 0, hq[0] + hq[3])
            d2 = down(2, 1, hq[0])
            d3 = down(3, 2, hq[1] - hq[3])
            d7 = down(7, 6, hq[2] + hq[3])
        last = (n // 2) % 2 == 1
        for hf, kh, o in ((0, 1, d2 + d4), (1, 0, d3 + d5), (1, 1, d1 - d2 + d3 + d6), (0, 0, d1 + d4 - d5 + d7)):
            rs = slice(hf * D + kh * KH, hf * D + (kh + 1) * KH)
            xo = xb[2 + slot, rs] + o
            if static:
                xb[2 + slot, rs] = xo
            else:
                o_v[blk, kh * KH:(kh + 1) * KH, hf * TH:(hf + 1) * TH] = xo.astype(bf16)
                if eager_out:
                    out_quadrant(blk, slot, hf, kh).start()
                nb = jnp.minimum(blk + 2, NT - 1)
                qn = q_v[2 * nb + hf, kh * KH:(kh + 1) * KH].astype(f32)
                xb[2 + slot, rs] = jnp.where(last, qn, xo)

    def products(c, hooks=None):
        hooks = hooks or {}
        count = [0]

        def mm(p):
            if count[0] in hooks:
                hooks[count[0]]()
            count[0] += 1
            b = b_operand(0, p) if c == 0 else _halves(bc_s[p])
            return _dot(_halves(agu[p, c * 8:(c + 1) * 8].reshape(B, KH)), b)

        rs = slice(c * B, (c + 1) * B)
        m2, m4 = mm(1), mm(3)
        hq[2, rs] = _act(m2 + m4)
        m5, m3 = mm(4), mm(2)
        hq[1, rs] = _act(m3 + m5)
        m1 = mm(0)
        m7 = mm(6)
        hq[0, rs] = _act(m1 + m4 - m5 + m7)
        m6 = mm(5)
        hq[3, rs] = _act(m1 - m2 + m3 + m6)

    def units0(lo, hi, inits):
        for s in range(lo, hi):
            table_unit(len(UNITS) * NSLOT + s, s in inits)

    def block(fn):
        pl.when(par[P_ZERO] == 0)(fn)

    start(group(0) + group(1))
    for s, (i, j) in enumerate([u for row in UNITS for u in row] + list(UNITS0)):
        tab[2 * s] = i
        tab[2 * s + 1] = j
    for i in range(8):
        par[i] = i // 4
    par[P_ZERO] = 0
    par[P_ZERO2] = 0
    for c in range(4):
        par[P_INT + c] = c
    ffwd, finv = _dft_mats()
    ffwd_v[...] = _words(ffwd)
    finv_v[...] = _words(finv)
    for t in range(3):
        g_s[t, 0] = jnp.zeros((D, B), f32)
    wait(group(0))
    start(group(2))
    sk = sk_v[...].astype(f32)
    dv = d_v[...].astype(f32).reshape(1, D)
    for j in range(5):
        row = sk[j:j + 1] if j < 4 else dv
        coef[j] = jnp.broadcast_to(row, (B, D)).T

    wait(group(1))
    start(group(8))
    conv_h(0)
    conv_u(0)
    conv_unit(0, 0, init=True)
    conv_inverse(0)
    wait(group(2))
    start(group(3))
    conv_h(1)
    conv_u(1)
    conv_unit(1, 0, init=True)
    conv_unit(1, 1)
    conv_inverse(1)
    wait(group(8))
    start(group(4))
    prep_gu(0)
    head(0)
    wait(group(3))
    start(group(5) + group(6))

    @block
    def _():
        products(0)
        for p in range(7):
            bc_s[p] = _words(b_operand(0, p))
        prep_gu(1)
        products(1)
        prep_gu(2)

    wait(group(4))

    @block
    def _():
        m = par[P_INT + 2]
        products(2, {1: lambda: conv_h(m), 3: lambda: conv_u(m)})
        prep_gu(3)
        units0(0, 4, (0, 3))
        products(3)
        conv_inverse(m)
        prep_gu(4)

    wait(group(5))
    start(late_copies(4) + group(7))

    @block
    def _():
        m = par[P_INT + 3]
        products(4, {1: lambda: conv_h(m), 3: lambda: conv_u(m)})
        prep_gu(5)
        units0(4, 9, (4,))
        products(5)
        prep_gu(6)
        load_q(1, 1)
        products(6)
        conv_inverse(m)

    wait(group(6))

    @block
    def _():
        prep_d()
        down_and_tail(0)

    def body(n, with_conv):
        slot = n % 2
        m = n + 3

        def unit(s):
            if with_conv:
                table_unit((n - 1) * NSLOT + s, (n < 4) if s == 0 else False)

        def mm(p):
            return _dot(_halves(agu[p].reshape(F // 2, KH)), b_operand(slot, p))

        if with_conv:
            wait(late_copies(m))
            conv_h(m)
        else:
            out_copy(item_block(n - 2), slot).wait()
        m2 = mm(1)
        if with_conv:
            conv_u(m)
        m5 = mm(4)
        unit(0)
        unit(1)
        m1 = mm(0)
        unit(2)
        unit(3)
        m4 = mm(3)
        hq[2] = _act(m2 + m4)
        unit(4)
        unit(5)
        m3 = mm(2)
        hq[1] = _act(m3 + m5)
        if with_conv:
            conv_inverse(m)
        m7 = mm(6)
        hq[0] = _act(m1 + m4 - m5 + m7)
        m6 = mm(5)
        hq[3] = _act(m1 - m2 + m3 + m6)
        down_and_tail(n, 2 if with_conv else 5, not with_conv)

        if with_conv:
            @pl.when((n // 2) % 2 == 1)
            def _():
                out_copy(item_block(n), slot).start()

    def body_conv(n, carry):
        body(n, True)
        return carry

    def body_plain(n, carry):
        body(n, False)
        return carry

    wait(group(7))
    start(late_copies(5) + late_copies(6) + late_copies(7))
    lax.fori_loop(1, 5, body_conv, 0)
    lax.fori_loop(5, 8, body_plain, 0)
    for slot in range(2):
        out_copy(NT - 2 + slot, slot).wait()


@jax.jit
def pallas_interleave_layers__ssm_conv_h3__geglu_ffn__prompt_kernel(A_q, A_k, A_v, A_shift_k, A_ssm_k, A_ssm_D, B_x, B_w_gate, B_w_up, B_w_down):
    hbm = pl.BlockSpec(memory_space=pl.ANY)
    out = pl.pallas_call(
        _kernel,
        in_specs=[hbm] * 9,
        out_specs=hbm,
        out_shape=jax.ShapeDtypeStruct((D, S), bf16),
        scratch_shapes=[
            pltpu.VMEM((NP, D, PW), bf16),
            pltpu.VMEM((NP, D, PW), bf16),
            pltpu.VMEM((NP, D, PW), bf16),
            pltpu.VMEM((NP, D, PW), bf16),
            pltpu.VMEM((D, F), bf16),
            pltpu.VMEM((D, F), bf16),
            pltpu.VMEM((D, F), bf16),
            pltpu.VMEM((4, D), bf16),
            pltpu.VMEM((D,), bf16),
            pltpu.VMEM((7, FH // 16, 2, 8, KH), u32),
            pltpu.VMEM((7, KH // 2, FH), u32),
            pltpu.VMEM((B // 2, 2 * B), u32),
            pltpu.VMEM((B, B), u32),
            pltpu.VMEM((5, D, B), f32),
            pltpu.VMEM((3, NB, D, B), f32),
            pltpu.VMEM((3, NB + 1, D, B), f32),
            pltpu.VMEM((2, D, B), f32),
            pltpu.VMEM((2, NB, D, B), f32),
            pltpu.VMEM((NB, D, B), f32),
            pltpu.VMEM((NT, D, TM), bf16),
            pltpu.VMEM((2, D, B), bf16),
            pltpu.VMEM((4, FH, TH), f32),
            pltpu.VMEM((4, FH, TH), f32),
            pltpu.VMEM((7, KH // 2, TH), u32),
            pltpu.SMEM((2 * (len(UNITS) * NSLOT + len(UNITS0)),), jnp.int32),
            pltpu.SMEM((P_INT + 4,), jnp.int32),
            pltpu.SemaphoreType.DMA((9,)),
            pltpu.SemaphoreType.DMA((4,)),
            pltpu.SemaphoreType.DMA((2,)),
        ],
        compiler_params=pltpu.CompilerParams(vmem_limit_bytes=110 * 1024 * 1024),
    )(A_q[0].T, A_k[0].T, A_v[0].T, A_shift_k.T, A_ssm_k, A_ssm_D, B_w_gate, B_w_up, B_w_down.T)
    return out.T[None]
```
